```python
import jax
import jax.numpy as jnp

def _softmax(x, axis=-1):
    return jax.nn.softmax(x, axis=axis)
def _gelu(x):
    return jax.nn.gelu(x, approximate=True)
def _silu(x):
    return jax.nn.silu(x)
def _sigmoid(x):
    return jax.nn.sigmoid(x)
def _layernorm(x, axis=-1, eps=1e-5):
    m = jnp.mean(x, axis=axis, keepdims=True)
    v = jnp.var(x, axis=axis, keepdims=True)
    return (x - m) / jnp.sqrt(v + eps)
def _scatter_add(tgt, idx, src, axis=0):
    return tgt.at[idx].add(src)
def _segment_sum(src, seg, n):
    return jax.ops.segment_sum(src, seg, n)
class _Rng:
    def __init__(self, key):
        self._k = key
    def _next(self):
        self._k, sub = jax.random.split(self._k)
        return sub
    def normal(self, shape):
        return jax.random.normal(self._next(), shape, dtype=jnp.bfloat16)
    def randint(self, lo, hi, shape):
        return jax.random.randint(self._next(), shape, lo, hi, dtype=jnp.int32)
    def uniform(self, shape, lo=0.0, hi=1.0):
        return jax.random.uniform(self._next(), shape, jnp.bfloat16, lo, hi)
    def permutation(self, n):
        return jax.random.permutation(self._next(), n)


kernel_name = 'concat_heads__ssm_conv_s5__sliding_local_dilated__prompt'

def setup_inputs():
    _rng = _Rng(jax.random.key(int.from_bytes(__import__("os").urandom(4), "little")))
    _w = (lambda a: (lambda t: t.astype(jnp.bfloat16) if jnp.issubdtype(t.dtype, jnp.floating) else t)(jnp.asarray(a)))
    def _A_setup():
        B, S, D = 1, 2048, 448
        P = D
        Lambda_re = -0.5 * jnp.exp((lambda *s: _rng.normal(s) * 0.05)(P))
        Lambda_im = (lambda *s: _rng.normal(s) * 0.05)(P) * 1.0
        B_re = (lambda *s: _rng.normal(s) * 0.05)(P, D) * (D ** -0.5)
        B_im = (lambda *s: _rng.normal(s) * 0.05)(P, D) * (D ** -0.5)
        C_re = (lambda *s: _rng.normal(s) * 0.05)(D, P) * (P ** -0.5)
        C_im = (lambda *s: _rng.normal(s) * 0.05)(D, P) * (P ** -0.5)
        log_dt = (lambda *s: _rng.normal(s) * 0.05)(P) * 0.3 - 2.0
        Dskip = (lambda *s: _rng.normal(s) * 0.05)(D)
        return {
            "x": _w((lambda *s: _rng.normal(s) * 0.05)(B, S, D)),
            "Lambda_re": _w(Lambda_re),
            "Lambda_im": _w(Lambda_im),
            "B_re": _w(B_re),
            "B_im": _w(B_im),
            "C_re": _w(C_re),
            "C_im": _w(C_im),
            "log_dt": _w(log_dt),
            "Dskip": _w(Dskip),
        }
    _A_in = _A_setup()

    def _B_setup():
        B, S, D = 1, 2048, 448
        return {
            "x": _w((lambda *s: _rng.normal(s) * 0.05)(B, S, D)),
            "wqkv": _w((lambda *s: _rng.normal(s) * 0.05)(D, 3 * D)),
            "wo": _w((lambda *s: _rng.normal(s) * 0.05)(D, D)),
        }
    _B_in = _B_setup()

    return {
        "A_x": _A_in["x"],
        "A_Lambda_re": _A_in["Lambda_re"],
        "A_Lambda_im": _A_in["Lambda_im"],
        "A_B_re": _A_in["B_re"],
        "A_B_im": _A_in["B_im"],
        "A_C_re": _A_in["C_re"],
        "A_C_im": _A_in["C_im"],
        "A_log_dt": _A_in["log_dt"],
        "A_Dskip": _A_in["Dskip"],
        "B_x": _B_in["x"],
        "B_wqkv": _B_in["wqkv"],
        "B_wo": _B_in["wo"],
    }

def reference(A_x, A_Lambda_re, A_Lambda_im, A_B_re, A_B_im, A_C_re, A_C_im, A_log_dt, A_Dskip, B_x, B_wqkv, B_wo):
    def _A_ref(x, Lambda_re, Lambda_im, B_re, B_im, C_re, C_im, log_dt, Dskip):
        Bsz, L, H = x.shape
        Lam = Lambda_re + 1j * Lambda_im
        Bmat = B_re + 1j * B_im
        Cmat = C_re + 1j * C_im
        dt = jnp.exp(log_dt)
        Lam_bar = jnp.exp(dt * Lam)
        B_bar = ((Lam_bar - 1.0) / Lam)[:, None] * Bmat
        Bu = jnp.einsum("bld,pd->blp", x + 0j, B_bar)
        h = jnp.zeros_like(Bu[:, 0, :])
        hs = []
        for t in range(L):
            h = Lam_bar[None, :] * h + Bu[:, t, :]
            hs.append(h)
        hseq = jnp.stack(hs, 1)
        y = 2.0 * jnp.einsum("blp,dp->bld", hseq, Cmat).real + x * Dskip[None, None, :]
        return y

    def _B_ref(x, wqkv, wo):
        B, S, D = x.shape
        H = 16; Dh = D // H
        W, dil = 8, 2
        qkv = (lambda x, *d: x.transpose(*d))((x @ wqkv).reshape(B, S, 3, H, Dh), 2, 0, 3, 1, 4)
        q, k, v = qkv[0], qkv[1], qkv[2]
        scale = Dh ** -0.5
        pos = jnp.arange(S)
        off = jnp.arange(W) * dil
        idx = pos[:, None] - off[None, :]
        mask = idx >= 0
        idx_c = jnp.where(mask, idx, 0).reshape(-1)
        kg = k[:, :, idx_c, :].reshape(B, H, S, W, Dh)
        vg = v[:, :, idx_c, :].reshape(B, H, S, W, Dh)
        logits = jnp.einsum("bhsd,bhswd->bhsw", q, kg) * scale
        logits = jnp.where(mask[None, None, :, :], logits, -1e9)
        attn = _softmax(logits, axis=-1)
        o = jnp.einsum("bhsw,bhswd->bhsd", attn, vg)
        return (lambda x, *d: x.transpose(*d))(o, 0, 2, 1, 3).reshape(B, S, D) @ wo

    a = _A_ref(A_x, A_Lambda_re, A_Lambda_im, A_B_re, A_B_im, A_C_re, A_C_im, A_log_dt, A_Dskip)
    b = _B_ref(B_x, B_wqkv, B_wo)
    return jnp.concatenate([a, b], axis=-1)
```

```python
import jax
import jax.numpy as jnp
from jax import lax
import jax.experimental.pallas as pl
import jax.experimental.pallas.tpu as pltpu

S = 2048
D = 448
H = 16
DH = D // H
WIN = 8
DIL = 2
TB = 256
NT = TB // 128
SEG = TB // 8
F32 = jnp.float32
BF16 = jnp.bfloat16
NT_DIMS = (((1,), (1,)), ((), ()))


def _cmul(ar, ai, br, bi):
    return ar * br - ai * bi, ar * bi + ai * br


def _kernel(xa_ref, xb_ref, lre_ref, lim_ref, ldt_ref, dsk_ref,
            bre_ref, bim_ref, cre_ref, cim_ref, wqkv_ref, wo_ref,
            out_ref,
            lam_ref, carry_ref, ccat_ref, wt_ref, wot_ref, dcol_ref, tmp_ref,
            u_ref, q_ref, k_ref, v_ref, ot_ref):
    step = pl.program_id(0)

    @pl.when(step == 0)
    def _setup():
        lre = lre_ref[...].astype(F32)
        lim = lim_ref[...].astype(F32)
        dt = jnp.exp(ldt_ref[...].astype(F32)).astype(BF16).astype(F32)
        mag = jnp.exp(dt * lre)
        ar = mag * jnp.cos(dt * lim)
        ai = mag * jnp.sin(dt * lim)
        den = lre * lre + lim * lim
        nr = ar - 1.0
        cr = 2.0 * (nr * lre + ai * lim) / den
        ci = 2.0 * (ai * lre - nr * lim) / den

        def tiles(x, sign):
            ts = [x[:, 128 * j:128 * (j + 1)] for j in range(3)]
            ts.append(jnp.concatenate([x[:, 384:], sign * x[:, 384:]], axis=1))
            return [jnp.broadcast_to(t, (8, 128)) for t in ts]

        sub = lax.broadcasted_iota(jnp.int32, (8, 128), 0)
        for j, (tr, ti) in enumerate(zip(tiles(ar, 1.0), tiles(ai, -1.0))):
            lam_ref[0, j] = tr
            lam_ref[1, j] = ti
            pr, pi = tr, ti
            n = 1
            while n < SEG:
                pr, pi = _cmul(pr, pi, pr, pi)
                n *= 2
            for lvl in range(3):
                lam_ref[2 + 2 * lvl, j] = jnp.where(sub >= (1 << lvl), pr, 0.0)
                lam_ref[3 + 2 * lvl, j] = jnp.where(sub >= (1 << lvl), pi, 0.0)
                pr, pi = _cmul(pr, pi, pr, pi)
        carry_ref[...] = jnp.zeros(carry_ref.shape, F32)

        c_re = cre_ref[...].astype(F32)
        c_im = cim_ref[...].astype(F32)
        e_re = c_re * cr - c_im * ci
        e_im = -(c_re * ci + c_im * cr)
        for j in range(3):
            ccat_ref[:, 256 * j:256 * j + 128] = e_re[:, 128 * j:128 * (j + 1)].astype(BF16)
            ccat_ref[:, 256 * j + 128:256 * (j + 1)] = e_im[:, 128 * j:128 * (j + 1)].astype(BF16)
        ccat_ref[:, 768:896] = jnp.concatenate([e_re[:, 384:], e_im[:, 384:]], axis=1).astype(BF16)

        dsk = jnp.broadcast_to(dsk_ref[...].astype(F32), (128, D))
        dcol_ref[...] = dsk.T

        for c in range(4):
            rows = 128 if c < 3 else 64
            wt = wqkv_ref[128 * c:128 * c + rows, :].astype(F32).T
            tmp_ref[c, :, 0:rows] = wt
        for c in range(4):
            rows = 128 if c < 3 else 64
            for m in range(3):
                for d in range(DH):
                    blk = tmp_ref[c, pl.ds(m * D + d, H, stride=DH), :]
                    wt_ref[m * D + d * H:m * D + (d + 1) * H, 128 * c:128 * c + rows] = (
                        blk[:, 0:rows].astype(BF16))
        for c in range(4):
            cols = 128 if c < 3 else 64
            tmp_ref[c, 0:D, 0:cols] = wo_ref[:, 128 * c:128 * c + cols].astype(F32)
        for c in range(4):
            cols = 128 if c < 3 else 64
            wp = jnp.concatenate(
                [tmp_ref[c, pl.ds(d, H, stride=DH), :] for d in range(DH)], axis=0)
            wot_ref[128 * c:128 * c + cols, :] = wp[:, 0:cols].T.astype(BF16)

        k_ref[0] = jnp.zeros((D, 128), F32)
        v_ref[0] = jnp.zeros((D, 128), F32)

    xb = xb_ref[...]
    qkv = jnp.dot(wt_ref[...], xb, preferred_element_type=F32)
    for j in range(NT):
        q_ref[j] = qkv[0:D, 128 * j:128 * (j + 1)]
        k_ref[j + 1] = qkv[D:2 * D, 128 * j:128 * (j + 1)]
        v_ref[j + 1] = qkv[2 * D:3 * D, 128 * j:128 * (j + 1)]

    xa_t = xa_ref[...]
    xa = xa_t.T
    for j in range(7):
        if j < 6:
            src = bre_ref if j % 2 == 0 else bim_ref
            w = src[128 * (j // 2):128 * (j // 2 + 1), :]
        else:
            w = jnp.concatenate([bre_ref[384:448, :], bim_ref[384:448, :]], axis=0)
        u = lax.dot_general(xa, w, NT_DIMS, preferred_element_type=F32)
        u_ref[j] = u
        if j == 6:
            u_ref[7] = pltpu.roll(u, 64, 1)

    lane = lax.broadcasted_iota(jnp.int32, (8, 128), 1)
    scale = DH ** -0.5

    def shifted(prev, cur, w):
        if w == 0:
            return cur
        s = DIL * w
        return pltpu.roll(jnp.where(lane >= 128 - s, prev, cur), s, 1)

    for j in range(NT):
        probs = []
        for hh in range(2):
            acc = [None] * WIN
            for d in range(DH):
                r = d * H + hh * 8
                qd = q_ref[j, r:r + 8, :]
                kc = k_ref[j + 1, r:r + 8, :]
                kp = k_ref[j, r:r + 8, :]
                for w in range(WIN):
                    t = qd * shifted(kp, kc, w)
                    acc[w] = t if acc[w] is None else acc[w] + t
            lg = [a * scale for a in acc]
            if j == 0:
                pos = lane + step * TB
                lg = [lg[0]] + [jnp.where(pos >= DIL * w, lg[w], -1e9) for w in range(1, WIN)]
            mx = lg[0]
            for w in range(1, WIN):
                mx = jnp.maximum(mx, lg[w])
            ex = [jnp.exp(l - mx) for l in lg]
            tot = ex[0]
            for w in range(1, WIN):
                tot = tot + ex[w]
            inv = 1.0 / tot
            probs.append([e * inv for e in ex])
        for d in range(DH):
            halves = []
            for hh in range(2):
                r = d * H + hh * 8
                vc = v_ref[j + 1, r:r + 8, :]
                vp = v_ref[j, r:r + 8, :]
                o = None
                for w in range(WIN):
                    t = probs[hh][w] * shifted(vp, vc, w)
                    o = t if o is None else o + t
                halves.append(o)
            ot_ref[d * H:(d + 1) * H, 128 * j:128 * (j + 1)] = (
                jnp.concatenate(halves, axis=0).astype(BF16))
    k_ref[0] = k_ref[NT]
    v_ref[0] = v_ref[NT]

    ob_t = jnp.dot(wot_ref[...], ot_ref[...], preferred_element_type=F32)

    sub = lax.broadcasted_iota(jnp.int32, (8, 128), 0)
    for p in range(4):
        ar = lam_ref[0, p]
        ai = lam_ref[1, p]

        def load(i):
            return (u_ref[2 * p, pl.ds(i, 8, stride=SEG), :],
                    u_ref[2 * p + 1, pl.ds(i, 8, stride=SEG), :])

        hr, hi = load(0)
        for i in range(1, SEG):
            ur, ui = load(i)
            hr, hi = ar * hr - ai * hi + ur, ar * hi + ai * hr + ui
        gr = pltpu.roll(jnp.where(sub == 7, carry_ref[2 * p], hr), 1, 0)
        gi = pltpu.roll(jnp.where(sub == 7, carry_ref[2 * p + 1], hi), 1, 0)
        for lvl in range(3):
            mr = lam_ref[2 + 2 * lvl, p]
            mi = lam_ref[3 + 2 * lvl, p]
            sr = pltpu.roll(gr, 1 << lvl, 0)
            si = pltpu.roll(gi, 1 << lvl, 0)
            gr, gi = gr + (mr * sr - mi * si), gi + (mr * si + mi * sr)
        hr, hi = gr, gi
        for i in range(SEG):
            ur, ui = load(i)
            hr, hi = ar * hr - ai * hi + ur, ar * hi + ai * hr + ui
            u_ref[2 * p, pl.ds(i, 8, stride=SEG), :] = hr
            if p < 3:
                u_ref[2 * p + 1, pl.ds(i, 8, stride=SEG), :] = hi
        carry_ref[2 * p] = hr
        carry_ref[2 * p + 1] = hi

    h = jnp.concatenate([u_ref[j].astype(BF16) for j in range(7)], axis=1)
    y_t = lax.dot_general(ccat_ref[...], h, NT_DIMS, preferred_element_type=F32)
    dcol = dcol_ref[...]
    y_t = y_t + xa_t.astype(F32) * jnp.concatenate([dcol] * NT, axis=1)
    out_ref[...] = jnp.concatenate([y_t, ob_t], axis=0).T


@jax.jit
def pallas_concat_heads__ssm_conv_s5__sliding_local_dilated__prompt_kernel(
    A_x, A_Lambda_re, A_Lambda_im, A_B_re, A_B_im, A_C_re, A_C_im, A_log_dt, A_Dskip,
    B_x, B_wqkv, B_wo,
):
    xa_t = jnp.swapaxes(A_x[0], 0, 1)
    xb_t = jnp.swapaxes(B_x[0], 0, 1)
    row = lambda v: v.reshape(1, D)
    full = lambda shape: pl.BlockSpec(shape, lambda i: (0,) * len(shape))
    xspec = pl.BlockSpec((D, TB), lambda i: (0, i))
    out = pl.pallas_call(
        _kernel,
        grid=(S // TB,),
        in_specs=[xspec, xspec] + [full((1, D))] * 4 + [full((D, D))] * 4
                 + [full((D, 3 * D)), full((D, D))],
        out_specs=pl.BlockSpec((TB, 2 * D), lambda i: (i, 0)),
        out_shape=jax.ShapeDtypeStruct((S, 2 * D), F32),
        scratch_shapes=[
            pltpu.VMEM((8, 4, 8, 128), F32),
            pltpu.VMEM((8, 8, 128), F32),
            pltpu.VMEM((D, 2 * D), BF16),
            pltpu.VMEM((3 * D, D), BF16),
            pltpu.VMEM((D, D), BF16),
            pltpu.VMEM((D, 128), F32),
            pltpu.VMEM((4, 3 * D, 128), F32),
            pltpu.VMEM((8, TB, 128), F32),
            pltpu.VMEM((NT, D, 128), F32),
            pltpu.VMEM((NT + 1, D, 128), F32),
            pltpu.VMEM((NT + 1, D, 128), F32),
            pltpu.VMEM((D, TB), BF16),
        ],
        compiler_params=pltpu.CompilerParams(
            dimension_semantics=("arbitrary",),
            vmem_limit_bytes=100 * 1024 * 1024,
        ),
    )(xa_t, xb_t, row(A_Lambda_re), row(A_Lambda_im), row(A_log_dt), row(A_Dskip),
      A_B_re, A_B_im, A_C_re, A_C_im, B_wqkv, B_wo)
    return out[None]
```

```python
import jax
import jax.numpy as jnp
from jax import lax
import jax.experimental.pallas as pl
import jax.experimental.pallas.tpu as pltpu

S = 2048
D = 448
H = 16
DH = D // H
WIN = 8
DIL = 2
TB = 256
NT = TB // 128
SEG = TB // 8
PITCH = SEG + 1
F32 = jnp.float32
BF16 = jnp.bfloat16
U32 = jnp.uint32
NT_DIMS = (((1,), (1,)), ((), ()))


def _cmul(ar, ai, br, bi):
    return ar * br - ai * bi, ar * bi + ai * br


def _pack(lo, hi):
    return pltpu.pack_elementwise([lo, hi], packed_dtype=BF16)


def _unpack(x):
    return [pltpu.unpack_elementwise(x, index=i, packed_dtype=BF16, unpacked_dtype=F32)
            for i in range(2)]


def _kernel(xa_ref, xb_ref, lre_ref, lim_ref, ldt_ref, dsk_ref,
            bre_ref, bim_ref, cre_ref, cim_ref, wqkv_ref, wo_ref,
            out_ref,
            lam_ref, carry_ref, ccat_ref, wt_ref, wot_ref, dcol_ref, tmp_ref,
            u_ref, q_ref, k_ref, v_ref, ot_ref):
    step = pl.program_id(0)

    @pl.when(step == 0)
    def _setup():
        lre = lre_ref[...].astype(F32)[None, :]
        lim = lim_ref[...].astype(F32)[None, :]
        dt = jnp.exp(ldt_ref[...].astype(F32)[None, :]).astype(BF16).astype(F32)
        mag = jnp.exp(dt * lre)
        ar = mag * jnp.cos(dt * lim)
        ai = mag * jnp.sin(dt * lim)
        den = lre * lre + lim * lim
        nr = ar - 1.0
        cr = 2.0 * (nr * lre + ai * lim) / den
        ci = 2.0 * (ai * lre - nr * lim) / den

        def tiles(x, sign):
            ts = [x[:, 128 * j:128 * (j + 1)] for j in range(3)]
            ts.append(jnp.concatenate([x[:, 384:], sign * x[:, 384:]], axis=1))
            return [jnp.broadcast_to(t, (8, 128)) for t in ts]

        sub = lax.broadcasted_iota(jnp.int32, (8, 128), 0)
        for j, (tr, ti) in enumerate(zip(tiles(ar, 1.0), tiles(ai, -1.0))):
            lam_ref[0, j] = tr
            lam_ref[1, j] = ti
            pr, pi = tr, ti
            n = 1
            while n < SEG:
                pr, pi = _cmul(pr, pi, pr, pi)
                n *= 2
            for lvl in range(3):
                lam_ref[2 + 2 * lvl, j] = jnp.where(sub >= (1 << lvl), pr, 0.0)
                lam_ref[3 + 2 * lvl, j] = jnp.where(sub >= (1 << lvl), pi, 0.0)
                pr, pi = _cmul(pr, pi, pr, pi)
        carry_ref[...] = jnp.zeros(carry_ref.shape, F32)

        c_re = cre_ref[...].astype(F32)
        c_im = cim_ref[...].astype(F32)
        e_re = c_re * cr - c_im * ci
        e_im = -(c_re * ci + c_im * cr)
        for j in range(3):
            ccat_ref[:, 256 * j:256 * j + 128] = e_re[:, 128 * j:128 * (j + 1)].astype(BF16)
            ccat_ref[:, 256 * j + 128:256 * (j + 1)] = e_im[:, 128 * j:128 * (j + 1)].astype(BF16)
        ccat_ref[:, 768:896] = jnp.concatenate([e_re[:, 384:], e_im[:, 384:]], axis=1).astype(BF16)

        dsk = jnp.broadcast_to(dsk_ref[...].astype(F32)[None, :], (128, D))
        dcol_ref[...] = dsk.T

        for c in range(4):
            rows = 128 if c < 3 else 64
            wt = wqkv_ref[128 * c:128 * c + rows, :].astype(F32).T
            tmp_ref[c, :, 0:rows] = wt
        for c in range(4):
            rows = 128 if c < 3 else 64
            for m in range(3):
                for d in range(DH):
                    blk = tmp_ref[c, pl.ds(m * D + d, H, stride=DH), :]
                    wt_ref[m * D + d * H:m * D + (d + 1) * H, 128 * c:128 * c + rows] = (
                        blk[:, 0:rows].astype(BF16))
        for c in range(4):
            cols = 128 if c < 3 else 64
            tmp_ref[c, 0:D, 0:cols] = wo_ref[:, 128 * c:128 * c + cols].astype(F32)
        for c in range(4):
            cols = 128 if c < 3 else 64
            wp = jnp.concatenate(
                [tmp_ref[c, pl.ds(d, H, stride=DH), :] for d in range(DH)], axis=0)
            wot_ref[128 * c:128 * c + cols, :] = wp[:, 0:cols].T.astype(BF16)

        k_ref[0] = jnp.zeros(k_ref.shape[1:], k_ref.dtype)
        v_ref[0] = jnp.zeros(v_ref.shape[1:], v_ref.dtype)

    xb = xb_ref[...]
    for m, dst in ((1, k_ref), (0, q_ref), (2, v_ref)):
        r = jnp.dot(wt_ref[m * D:(m + 1) * D, :], xb, preferred_element_type=F32)
        for j in range(NT):
            rj = r[:, 128 * j:128 * (j + 1)]
            if m == 0:
                dst[j] = rj
            else:
                for d in range(DH):
                    dst[j + 1, 8 * d:8 * d + 8, :] = _pack(rj[16 * d:16 * d + 8], rj[16 * d + 8:16 * d + 16])

    xa = xa_ref[...].T
    bcat = jnp.concatenate(
        [(bre_ref if j % 2 == 0 else bim_ref)[128 * (j // 2):128 * (j // 2 + 1), :] for j in range(6)]
        + [bre_ref[384:448, :], bim_ref[384:448, :]], axis=0)
    u = lax.dot_general(xa, bcat, NT_DIMS, preferred_element_type=F32)
    for j in range(8):
        uj = u[:, 128 * j:128 * (j + 1)] if j < 7 else pltpu.roll(u[:, 768:896], 64, 1)
        for s in range(8):
            u_ref[j, s * PITCH:s * PITCH + SEG, :] = uj[s * SEG:(s + 1) * SEG]

    lane = lax.broadcasted_iota(jnp.int32, (8, 128), 1)
    scale = DH ** -0.5

    def shifted(prev, cur, w):
        if w == 0:
            return _unpack(cur)
        s = DIL * w
        return _unpack(pltpu.roll(jnp.where(lane >= 128 - s, prev, cur), s, 1))

    for j in range(NT):
        acc = [[None] * WIN for _ in range(2)]
        for d in range(DH):
            qd = [q_ref[j, 16 * d + 8 * hh:16 * d + 8 * hh + 8, :] for hh in range(2)]
            kc = k_ref[j + 1, 8 * d:8 * d + 8, :]
            kp = k_ref[j, 8 * d:8 * d + 8, :]
            for w in range(WIN):
                ks = shifted(kp, kc, w)
                for hh in range(2):
                    t = qd[hh] * ks[hh]
                    acc[hh][w] = t if d == 0 else acc[hh][w] + t
        probs = []
        for hh in range(2):
            lg = [a * scale for a in acc[hh]]
            if j == 0:
                pos = lane + step * TB
                lg = [lg[0]] + [jnp.where(pos >= DIL * w, lg[w], -1e9) for w in range(1, WIN)]
            mx = lg[0]
            for w in range(1, WIN):
                mx = jnp.maximum(mx, lg[w])
            ex = [jnp.exp(l - mx) for l in lg]
            tot = ex[0]
            for w in range(1, WIN):
                tot = tot + ex[w]
            inv = 1.0 / tot
            probs.append([e * inv for e in ex])
        for d in range(DH):
            vc = v_ref[j + 1, 8 * d:8 * d + 8, :]
            vp = v_ref[j, 8 * d:8 * d + 8, :]
            o = [None, None]
            for w in range(WIN):
                vs = shifted(vp, vc, w)
                for hh in range(2):
                    t = probs[hh][w] * vs[hh]
                    o[hh] = t if w == 0 else o[hh] + t
            ot_ref[d * H:(d + 1) * H, 128 * j:128 * (j + 1)] = (
                jnp.concatenate(o, axis=0).astype(BF16))
    k_ref[0] = k_ref[NT]
    v_ref[0] = v_ref[NT]

    ob_t = jnp.dot(wot_ref[...], ot_ref[...], preferred_element_type=F32)
    out_ref[:, 512:896] = ob_t[64:448].T

    sub = lax.broadcasted_iota(jnp.int32, (8, 128), 0)
    for p in range(4):
        ar = lam_ref[0, p]
        ai = lam_ref[1, p]

        def load(i):
            return (u_ref[2 * p, pl.ds(i, 8, stride=PITCH), :],
                    u_ref[2 * p + 1, pl.ds(i, 8, stride=PITCH), :])

        hr, hi = load(0)
        for i in range(1, SEG):
            ur, ui = load(i)
            hr, hi = ar * hr + (ur - ai * hi), ar * hi + (ai * hr + ui)
        gr = pltpu.roll(jnp.where(sub == 7, carry_ref[2 * p], hr), 1, 0)
        gi = pltpu.roll(jnp.where(sub == 7, carry_ref[2 * p + 1], hi), 1, 0)
        for lvl in range(3):
            mr = lam_ref[2 + 2 * lvl, p]
            mi = lam_ref[3 + 2 * lvl, p]
            sr = pltpu.roll(gr, 1 << lvl, 0)
            si = pltpu.roll(gi, 1 << lvl, 0)
            gr, gi = gr + (mr * sr - mi * si), gi + (mr * si + mi * sr)
        hr, hi = gr, gi
        for i in range(SEG):
            ur, ui = load(i)
            hr, hi = ar * hr + (ur - ai * hi), ar * hi + (ai * hr + ui)
            u_ref[2 * p, pl.ds(i, 8, stride=PITCH), :] = hr
            if p < 3:
                u_ref[2 * p + 1, pl.ds(i, 8, stride=PITCH), :] = hi
        carry_ref[2 * p] = hr
        carry_ref[2 * p + 1] = hi

    h = jnp.concatenate(
        [jnp.concatenate([u_ref[j, s * PITCH:s * PITCH + SEG, :] for s in range(8)], axis=0).astype(BF16)
         for j in range(7)], axis=1)
    y_t = lax.dot_general(ccat_ref[...], h, NT_DIMS, preferred_element_type=F32)
    dcol = dcol_ref[...]
    y_t = y_t + xa_ref[...].astype(F32) * jnp.concatenate([dcol] * NT, axis=1)
    out_ref[:, 0:512] = jnp.concatenate([y_t, ob_t[0:64]], axis=0).T


@jax.jit
def pallas_concat_heads__ssm_conv_s5__sliding_local_dilated__prompt_kernel(
    A_x, A_Lambda_re, A_Lambda_im, A_B_re, A_B_im, A_C_re, A_C_im, A_log_dt, A_Dskip,
    B_x, B_wqkv, B_wo,
):
    xa_t = jnp.swapaxes(A_x[0], 0, 1)
    xb_t = jnp.swapaxes(B_x[0], 0, 1)
    full = lambda shape: pl.BlockSpec(shape, lambda i: (0,) * len(shape))
    xspec = pl.BlockSpec((D, TB), lambda i: (0, i))
    out = pl.pallas_call(
        _kernel,
        grid=(S // TB,),
        in_specs=[xspec, xspec] + [full((D,))] * 4 + [full((D, D))] * 4
                 + [full((D, 3 * D)), full((D, D))],
        out_specs=pl.BlockSpec((TB, 2 * D), lambda i: (i, 0)),
        out_shape=jax.ShapeDtypeStruct((S, 2 * D), F32),
        scratch_shapes=[
            pltpu.VMEM((8, 4, 8, 128), F32),
            pltpu.VMEM((8, 8, 128), F32),
            pltpu.VMEM((D, 2 * D), BF16),
            pltpu.VMEM((3 * D, D), BF16),
            pltpu.VMEM((D, D), BF16),
            pltpu.VMEM((D, 128), F32),
            pltpu.VMEM((4, 3 * D, 128), F32),
            pltpu.VMEM((8, 8 * PITCH, 128), F32),
            pltpu.VMEM((NT, D, 128), F32),
            pltpu.VMEM((NT + 1, D // 2, 128), U32),
            pltpu.VMEM((NT + 1, D // 2, 128), U32),
            pltpu.VMEM((D, TB), BF16),
        ],
        compiler_params=pltpu.CompilerParams(
            dimension_semantics=("arbitrary",),
            vmem_limit_bytes=100 * 1024 * 1024,
        ),
    )(xa_t, xb_t, A_Lambda_re, A_Lambda_im, A_log_dt, A_Dskip,
      A_B_re, A_B_im, A_C_re, A_C_im, B_wqkv, B_wo)
    return out[None]
```

```python
import jax
import jax.numpy as jnp
from jax import lax
import jax.experimental.pallas as pl
import jax.experimental.pallas.tpu as pltpu

S = 2048
D = 448
DP = 512
H = 16
DH = D // H
WIN = 8
DIL = 2
TB = 512
NB = S // TB
NT = TB // 128
SB = 256
NS = TB // SB
SEG = SB // 8
PITCH = SEG + 1
F32 = jnp.float32
BF16 = jnp.bfloat16
U32 = jnp.uint32
NT_DIMS = (((1,), (1,)), ((), ()))


def _cmul(ar, ai, br, bi):
    return ar * br - ai * bi, ar * bi + ai * br


def _pack(lo, hi):
    return pltpu.pack_elementwise([lo, hi], packed_dtype=BF16)


def _unpack(x):
    return [pltpu.unpack_elementwise(x, index=i, packed_dtype=BF16, unpacked_dtype=F32)
            for i in range(2)]


def _words(x):
    return pltpu.bitcast(x.astype(BF16), U32)


def _halves(w):
    return pltpu.bitcast(w, BF16)


def _pad_lanes(x):
    if x.shape[1] == 128:
        return x
    return jnp.concatenate([x, jnp.zeros((x.shape[0], 128 - x.shape[1]), x.dtype)], axis=1)


def _kernel(xa_hbm, xb_hbm, lre_hbm, lim_hbm, ldt_hbm, dsk_hbm,
            bre_hbm, bim_hbm, cre_hbm, cim_hbm, wqkv_hbm, wo_hbm,
            out_hbm,
            xa_ref, xb_ref, lre_ref, lim_ref, ldt_ref, dsk_ref,
            bre_ref, bim_ref, cre_ref, cim_ref, wqkv_ref, wo_ref,
            lam_ref, carry_ref, ccat_ref, wt_ref, wot_ref, dcol_ref, tmp_ref, tmp2_ref,
            xt_ref, u_ref, h_ref, q_ref, k_ref, v_ref, ot_ref, y_ref, out_ref, isem, osem):
    copies = {}

    def fetch(name, src, dst):
        cp = pltpu.make_async_copy(src, dst, isem.at[2 * NB + len(copies)])
        cp.start()
        copies[name] = cp

    def wait(*names):
        for n in names:
            copies[n].wait()

    def tokens(b):
        return pl.ds(b * TB if isinstance(b, int) else pl.multiple_of(b * TB, TB), TB)

    def x_copy(which, b):
        hbm, ref = ((xa_hbm, xa_ref), (xb_hbm, xb_ref))[which]
        return pltpu.make_async_copy(hbm.at[:, tokens(b)], ref.at[b], isem.at[which * NB + b])

    def out_copy(b):
        return pltpu.make_async_copy(out_ref.at[b], out_hbm.at[tokens(b), :], osem.at[b])

    def tail_copy(j, part):
        cols = (pl.ds(512, 384), pl.ds(0, 512))[part]
        return pltpu.make_async_copy(
            out_ref.at[NB - 1, pl.ds(128 * j, 128), cols],
            out_hbm.at[pl.ds((NB - 1) * TB + 128 * j, 128), cols],
            osem.at[NB - 1 + 2 * j + part])

    def w_cols(lo, hi):
        return wqkv_hbm.at[:, pl.ds(lo, hi - lo)], wqkv_ref.at[:, pl.ds(lo, hi - lo)]

    x_copy(0, 0).start()
    fetch("bre", bre_hbm, bre_ref)
    fetch("bim", bim_hbm, bim_ref)
    fetch("lre", lre_hbm, lre_ref)
    fetch("lim", lim_hbm, lim_ref)
    fetch("ldt", ldt_hbm, ldt_ref)
    fetch("dsk", dsk_hbm, dsk_ref)
    fetch("wq", *w_cols(0, 512))
    fetch("wk", *w_cols(512, 896))
    x_copy(1, 0).start()
    fetch("wv", *w_cols(896, 1344))
    fetch("cre", cre_hbm, cre_ref)
    fetch("cim", cim_hbm, cim_ref)
    fetch("wo", wo_hbm, wo_ref)
    x_copy(0, 1).start()
    x_copy(1, 1).start()

    sub = lax.broadcasted_iota(jnp.int32, (8, 128), 0)
    lane = lax.broadcasted_iota(jnp.int32, (8, 128), 1)

    def setup_lambda():
        lre = lre_ref[...].astype(F32)[None, :]
        lim = lim_ref[...].astype(F32)[None, :]
        dt = jnp.exp(ldt_ref[...].astype(F32)[None, :]).astype(BF16).astype(F32)
        mag = jnp.exp(dt * lre)
        ar = mag * jnp.cos(dt * lim)
        ai = mag * jnp.sin(dt * lim)
        den = lre * lre + lim * lim
        nr = ar - 1.0
        cr = 2.0 * (nr * lre + ai * lim) / den
        ci = 2.0 * (ai * lre - nr * lim) / den

        def tiles(x, sign):
            ts = [x[:, 128 * j:128 * (j + 1)] for j in range(3)]
            ts.append(jnp.concatenate([x[:, 384:], sign * x[:, 384:]], axis=1))
            return [jnp.broadcast_to(t, (8, 128)) for t in ts]

        for j, (tr, ti) in enumerate(zip(tiles(ar, 1.0), tiles(ai, -1.0))):
            lam_ref[0, j] = tr
            lam_ref[1, j] = ti
            pr, pi = tr, ti
            n = 1
            while n < SEG:
                pr, pi = _cmul(pr, pi, pr, pi)
                n *= 2
            for lvl in range(3):
                lam_ref[2 + 2 * lvl, j] = jnp.where(sub >= (1 << lvl), pr, 0.0)
                lam_ref[3 + 2 * lvl, j] = jnp.where(sub >= (1 << lvl), pi, 0.0)
                pr, pi = _cmul(pr, pi, pr, pi)
        carry_ref[...] = jnp.zeros(carry_ref.shape, F32)
        dsk = jnp.broadcast_to(dsk_ref[...].astype(F32)[None, :], (128, D))
        dcol_ref[...] = dsk.T
        return cr, ci

    def setup_c(cr, ci):
        for r in range(0, D, 32):
            c_re = cre_ref[r:r + 32, :].astype(F32)
            c_im = cim_ref[r:r + 32, :].astype(F32)
            e_re = c_re * cr - c_im * ci
            e_im = -(c_re * ci + c_im * cr)
            rows = slice(r // 2, r // 2 + 16)
            for j in range(3):
                ccat_ref[rows, 256 * j:256 * j + 128] = _words(e_re[:, 128 * j:128 * (j + 1)])
                ccat_ref[rows, 256 * j + 128:256 * (j + 1)] = _words(e_im[:, 128 * j:128 * (j + 1)])
            ccat_ref[rows, 768:896] = _words(jnp.concatenate([e_re[:, 384:], e_im[:, 384:]], axis=1))

    def setup_w(m):
        lo, hi = ((0, 512), (512, 896), (896, 1344))[m]
        for n in range(lo, hi, 128):
            n1 = min(n + 128, hi)
            for c in range(4):
                rows = 128 if c < 3 else 64
                tmp_ref[c, n:n1, :] = _pad_lanes(
                    wqkv_ref[128 * c:128 * c + rows, n:n1].astype(F32).T)
        for d in range(DH):
            for c in range(4):
                r = (m * D + d * H) // 2
                wt_ref[r:r + 8, 128 * c:128 * (c + 1)] = _words(
                    tmp_ref[c, pl.ds(m * D + d, H, stride=DH), :])

    def setup_wo():
        for c in range(4):
            cols = 128 if c < 3 else 64
            tmp2_ref[c] = _pad_lanes(wo_ref[:, 128 * c:128 * c + cols].astype(F32))
        for c in range(4):
            cols = 128 if c < 3 else 64
            wp = jnp.concatenate(
                [tmp2_ref[c, pl.ds(d, H, stride=DH), :] for d in range(DH)]
                + [jnp.zeros((DP - D, 128), F32)], axis=0)
            wot_ref[64 * c:64 * c + cols // 2, :] = _words(wp.T[0:cols])

    def transpose_x(b):
        xt_ref[...] = pltpu.bitcast(xa_ref[b].T, U32)

    def ssm_in(tiles):
        for j in tiles:
            if j == 6:
                w = jnp.concatenate([bre_ref[384:448, :], bim_ref[384:448, :]], axis=0)
            else:
                w = (bim_ref if j % 2 else bre_ref)[128 * (j // 2):128 * (j // 2 + 1), :]
            u = lax.dot_general(_halves(xt_ref[...]), w, NT_DIMS, preferred_element_type=F32)
            for jj, uj in ((j, u), (7, pltpu.roll(u, 64, 1))) if j == 6 else ((j, u),):
                for g in range(TB // SEG):
                    s, r = divmod(g, 8)
                    u_ref[s, jj, r * PITCH:r * PITCH + SEG, :] = uj[g * SEG:(g + 1) * SEG]

    def scan(s, pairs=(3, 0, 1, 2)):
        lam = {p: (lam_ref[0, p], lam_ref[1, p]) for p in pairs}

        def step(i, h):
            new = {}
            for p in pairs:
                ur = u_ref[s, 2 * p, pl.ds(i, 8, stride=PITCH), :]
                ui = u_ref[s, 2 * p + 1, pl.ds(i, 8, stride=PITCH), :]
                if h is not None:
                    (ar, ai), (hr, hi) = lam[p], h[p]
                    ur, ui = ar * hr + (ur - ai * hi), ar * hi + (ai * hr + ui)
                new[p] = (ur, ui)
            return new

        h = None
        for i in range(SEG):
            h = step(i, h)
        for p in pairs:
            gr = pltpu.roll(jnp.where(sub == 7, carry_ref[2 * p], h[p][0]), 1, 0)
            gi = pltpu.roll(jnp.where(sub == 7, carry_ref[2 * p + 1], h[p][1]), 1, 0)
            for lvl in range(3):
                mr = lam_ref[2 + 2 * lvl, p]
                mi = lam_ref[3 + 2 * lvl, p]
                sr = pltpu.roll(gr, 1 << lvl, 0)
                si = pltpu.roll(gi, 1 << lvl, 0)
                gr, gi = gr + (mr * sr - mi * si), gi + (mr * si + mi * sr)
            h[p] = (gr, gi)
        for i in range(SEG):
            h = step(i, h)
            for p in pairs:
                for t in range(2 * p, min(2 * p + 2, 7)):
                    h_ref[s, t, pl.ds(i, 8, stride=PITCH), :] = h[p][t % 2]
        for p in pairs:
            carry_ref[2 * p], carry_ref[2 * p + 1] = h[p]

    def ssm_out(b, j):
        s, g0 = divmod(j * (128 // SEG), 8)
        h = jnp.concatenate(
            [jnp.concatenate([h_ref[s, t, g * PITCH:g * PITCH + SEG, :]
                              for g in range(g0, g0 + 128 // SEG)], axis=0).astype(BF16)
             for t in range(7)], axis=1)
        y_t = lax.dot_general(_halves(ccat_ref[...]), h, NT_DIMS, preferred_element_type=F32)
        return y_t + xa_ref[b, :, 128 * j:128 * (j + 1)].astype(F32) * dcol_ref[...]

    kpad = jnp.zeros((DP - D, 128), BF16)

    def proj(b, m, j):
        xb = jnp.concatenate([xb_ref[b, :, 128 * j:128 * (j + 1)], kpad], axis=0)
        r = jnp.dot(_halves(wt_ref[m * D // 2:(m + 1) * D // 2, :]), xb, preferred_element_type=F32)
        if m == 0:
            q_ref[j] = r
        else:
            dst = k_ref if m == 1 else v_ref
            for d in range(DH):
                dst[j + 1, 8 * d:8 * d + 8, :] = _pack(r[16 * d:16 * d + 8], r[16 * d + 8:16 * d + 16])

    def shifted(prev, cur, w):
        if w == 0:
            return _unpack(cur)
        s = DIL * w
        return _unpack(pltpu.roll(jnp.where(lane >= 128 - s, prev, cur), s, 1))

    def scores(j, first):
        acc = [[None] * WIN for _ in range(2)]
        for w0 in range(0, WIN, 4):
            for d in range(DH):
                qd = [q_ref[j, 16 * d + 8 * hh:16 * d + 8 * hh + 8, :] for hh in range(2)]
                kc = k_ref[j + 1, 8 * d:8 * d + 8, :]
                kp = k_ref[j, 8 * d:8 * d + 8, :]
                for w in range(w0, w0 + 4):
                    ks = shifted(kp, kc, w)
                    for hh in range(2):
                        t = qd[hh] * ks[hh]
                        acc[hh][w] = t if d == 0 else acc[hh][w] + t
        probs = []
        for hh in range(2):
            lg = [a * (DH ** -0.5) for a in acc[hh]]
            if first:
                lg = [lg[0]] + [jnp.where(lane >= DIL * w, lg[w], -1e9) for w in range(1, WIN)]
            mx = lg[0]
            for w in range(1, WIN):
                mx = jnp.maximum(mx, lg[w])
            ex = [jnp.exp(l - mx) for l in lg]
            tot = ex[0]
            for w in range(1, WIN):
                tot = tot + ex[w]
            inv = 1.0 / tot
            probs.append([e * inv for e in ex])
        return probs

    def values(j, probs):
        for d in range(DH):
            vc = v_ref[j + 1, 8 * d:8 * d + 8, :]
            vp = v_ref[j, 8 * d:8 * d + 8, :]
            o = [None, None]
            for w in range(WIN):
                vs = shifted(vp, vc, w)
                for hh in range(2):
                    t = probs[hh][w] * vs[hh]
                    o[hh] = t if w == 0 else o[hh] + t
            ot_ref[j, 8 * d:8 * d + 8, :] = _words(jnp.concatenate(o, axis=0))

    def keep_halo():
        k_ref[0] = k_ref[NT]
        v_ref[0] = v_ref[NT]

    def attn_out(j):
        o_t = jnp.concatenate([_halves(ot_ref[j]), kpad], axis=0)
        return jnp.dot(_halves(wot_ref[...]), o_t, preferred_element_type=F32)

    def finish(b):
        for j in range(NT):
            out_ref[b, 128 * j:128 * (j + 1), :] = jnp.concatenate(
                [y_ref[j], attn_out(j)], axis=0).T
        out_copy(b).start()

    def front(b):
        transpose_x(b)
        ssm_in((6, 0, 1, 2, 3, 4, 5))
        for j in range(NT):
            for m in range(3):
                proj(b, m, j)
            if j < NS:
                scan(j)
            values(j, scores(j, False))
        keep_halo()

    k_ref[0] = jnp.zeros(k_ref.shape[1:], k_ref.dtype)
    v_ref[0] = jnp.zeros(v_ref.shape[1:], v_ref.dtype)
    x_copy(0, 0).wait()
    transpose_x(0)
    wait("bre")
    ssm_in((0, 2, 4))
    wait("bim", "lre", "lim", "ldt", "dsk", "wq")
    cr, ci = setup_lambda()
    ssm_in((6, 1, 3, 5))
    for s in range(NS):
        scan(s, (3, 0))
    setup_w(0)
    x_copy(1, 0).wait()
    wait("wk", "wv")
    for j in range(NT):
        proj(0, 0, j)
    setup_w(1)
    for j in range(NT):
        proj(0, 1, j)
    for s in range(NS):
        scan(s, (1, 2))
    setup_w(2)
    probs = [scores(0, True)]
    wait("cre", "cim", "wo")
    for j in range(NT):
        proj(0, 2, j)
    setup_c(cr, ci)
    for j in range(NT):
        y_ref[j] = ssm_out(0, j)
        values(j, probs[0] if j == 0 else scores(j, False))
    keep_halo()
    setup_wo()

    @pl.loop(1, NB - 1)
    def _(b):
        x_copy(0, b + 1).start()
        x_copy(1, b + 1).start()
        x_copy(0, b).wait()
        x_copy(1, b).wait()
        finish(b - 1)
        front(b)
        for j in range(NT):
            y_ref[j] = ssm_out(b, j)

    last = NB - 1
    x_copy(0, last).wait()
    x_copy(1, last).wait()
    finish(last - 1)
    front(last)
    for j in range(NT):
        rows = slice(128 * j, 128 * (j + 1))
        ob_t = attn_out(j)
        out_ref[last, rows, 512:896] = ob_t[64:448].T
        tail_copy(j, 0).start()
        out_ref[last, rows, 0:512] = jnp.concatenate([ssm_out(last, j), ob_t[0:64]], axis=0).T
        tail_copy(j, 1).start()
    for b in range(NB - 1):
        out_copy(b).wait()
    for j in range(NT):
        tail_copy(j, 0).wait()
        tail_copy(j, 1).wait()


@jax.jit
def pallas_concat_heads__ssm_conv_s5__sliding_local_dilated__prompt_kernel(
    A_x, A_Lambda_re, A_Lambda_im, A_B_re, A_B_im, A_C_re, A_C_im, A_log_dt, A_Dskip,
    B_x, B_wqkv, B_wo,
):
    xa_t = jnp.swapaxes(A_x[0], 0, 1)
    xb_t = jnp.swapaxes(B_x[0], 0, 1)
    hbm = pl.BlockSpec(memory_space=pltpu.HBM)
    vm = pltpu.VMEM
    out = pl.pallas_call(
        _kernel,
        in_specs=[hbm] * 12,
        out_specs=hbm,
        out_shape=jax.ShapeDtypeStruct((S, 2 * D), F32),
        scratch_shapes=[
            vm((NB, D, TB), BF16), vm((NB, D, TB), BF16),
            vm((D,), BF16), vm((D,), BF16), vm((D,), BF16), vm((D,), BF16),
            vm((D, D), BF16), vm((D, D), BF16), vm((D, D), BF16), vm((D, D), BF16),
            vm((D, 3 * D), BF16), vm((D, D), BF16),
            vm((8, 4, 8, 128), F32),
            vm((8, 8, 128), F32),
            vm((D // 2, 2 * D), U32),
            vm((3 * D // 2, DP), U32),
            vm((D // 2, DP), U32),
            vm((D, 128), F32),
            vm((4, 3 * D, 128), F32),
            vm((4, D, 128), F32),
            vm((TB // 2, D), U32),
            vm((NS, 8, 8 * PITCH, 128), F32),
            vm((NS, 7, 8 * PITCH, 128), F32),
            vm((NT, D, 128), F32),
            vm((NT + 1, D // 2, 128), U32),
            vm((NT + 1, D // 2, 128), U32),
            vm((NT, D // 2, 128), U32),
            vm((NT, D, 128), F32),
            vm((NB, TB, 2 * D), F32),
            pltpu.SemaphoreType.DMA((2 * NB + 12,)),
            pltpu.SemaphoreType.DMA((NB - 1 + 2 * NT,)),
        ],
        compiler_params=pltpu.CompilerParams(vmem_limit_bytes=100 * 1024 * 1024),
    )(xa_t, xb_t, A_Lambda_re, A_Lambda_im, A_log_dt, A_Dskip,
      A_B_re, A_B_im, A_C_re, A_C_im, B_wqkv, B_wo)
    return out[None]
```

```python
import jax
import jax.numpy as jnp
import numpy as np
from jax import lax
import jax.experimental.pallas as pl
import jax.experimental.pallas.tpu as pltpu

S = 2048
D = 448
DP = 512
H = 16
DH = D // H
WIN = 8
DIL = 2
TB = 512
NB = S // TB
NT = TB // 128
SB = 256
NS = TB // SB
SEG = SB // 8
PITCH = SEG + 1
W_COLS = ((0, 384), (384, 896), (896, 3 * D))
F32 = jnp.float32
BF16 = jnp.bfloat16
U32 = jnp.uint32
NT_DIMS = (((1,), (1,)), ((), ()))


def _cmul(ar, ai, br, bi):
    return ar * br - ai * bi, ar * bi + ai * br


def _pack(lo, hi):
    return pltpu.pack_elementwise([lo, hi], packed_dtype=BF16)


def _unpack(x):
    return [pltpu.unpack_elementwise(x, index=i, packed_dtype=BF16, unpacked_dtype=F32)
            for i in range(2)]


def _words(x):
    return pltpu.bitcast(x.astype(BF16), U32)


def _halves(w):
    return pltpu.bitcast(w, BF16)


def _pad_lanes(x):
    if x.shape[1] == 128:
        return x
    return jnp.concatenate([x, jnp.zeros((x.shape[0], 128 - x.shape[1]), x.dtype)], axis=1)


def _kernel(xa_hbm, xb_hbm, lre_hbm, lim_hbm, ldt_hbm, dsk_hbm,
            bre_hbm, bim_hbm, cre_hbm, cim_hbm, wqkv_hbm, wo_hbm,
            out_hbm,
            xa_ref, xb_ref, lre_ref, lim_ref, ldt_ref, dsk_ref,
            bre_ref, bim_ref, cre_ref, cim_ref, wqkv_ref, wo_ref,
            lam_ref, carry_ref, ccat_ref, wt_ref, wot_ref, dcol_ref, tmp_ref, tmp2_ref,
            xt_ref, u_ref, h_ref, q_ref, k_ref, v_ref, ot_ref, y_ref, out_ref, spare_ref, isem, osem):
    copies = {}

    def fetch(group, src, dst):
        cp = pltpu.make_async_copy(src, dst, isem.at[group])
        cp.start()
        copies.setdefault(group, []).append(cp)

    def wait(group):
        for cp in copies[group]:
            cp.wait()

    def tokens(b):
        return pl.ds(b * TB if isinstance(b, int) else pl.multiple_of(b * TB, TB), TB)

    def x_copies(b):
        return [pltpu.make_async_copy(hbm.at[:, tokens(b)], ref.at[b], isem.at[4 + b])
                for hbm, ref in ((xa_hbm, xa_ref), (xb_hbm, xb_ref))]

    def out_copy(b):
        return pltpu.make_async_copy(out_ref.at[tokens(b)], out_hbm.at[tokens(b), :], osem)

    def tail_copy(j, lo, hi):
        rows, cols = pl.ds((NB - 1) * TB + 128 * j, 128), pl.ds(lo, hi - lo)
        return pltpu.make_async_copy(out_ref.at[rows, cols], out_hbm.at[rows, cols], osem)

    def w_cols(lo, hi):
        return wqkv_hbm.at[:, pl.ds(lo, hi - lo)], wqkv_ref.at[:, pl.ds(lo, hi - lo)]

    def rows_of(hbm, ref, lo, hi):
        return hbm.at[pl.ds(lo, hi - lo)], ref.at[pl.ds(lo, hi - lo)]

    fetch(0, xa_hbm.at[:, tokens(0)], xa_ref.at[0])
    fetch(1, lre_hbm, lre_ref)
    fetch(1, lim_hbm, lim_ref)
    fetch(1, ldt_hbm, ldt_ref)
    fetch(1, dsk_hbm, dsk_ref)
    fetch(1, *rows_of(bre_hbm, bre_ref, 384, D))
    fetch(1, *rows_of(bim_hbm, bim_ref, 384, D))
    fetch(1, *rows_of(bre_hbm, bre_ref, 0, 256))
    fetch(1, *rows_of(bim_hbm, bim_ref, 0, 128))
    fetch(2, *rows_of(bre_hbm, bre_ref, 256, 384))
    fetch(2, *rows_of(bim_hbm, bim_ref, 128, 384))
    fetch(2, *w_cols(*W_COLS[1]))
    fetch(2, *w_cols(*W_COLS[0]))
    fetch(3, xb_hbm.at[:, tokens(0)], xb_ref.at[0])
    fetch(3, *w_cols(*W_COLS[2]))
    fetch(4, cre_hbm, cre_ref)
    fetch(4, cim_hbm, cim_ref)
    fetch(4, wo_hbm, wo_ref)
    for cp in x_copies(1):
        cp.start()

    sub = lax.broadcasted_iota(jnp.int32, (8, 128), 0)
    lane = lax.broadcasted_iota(jnp.int32, (8, 128), 1)

    def setup_lambda():
        lre = lre_ref[...].astype(F32)[None, :]
        lim = lim_ref[...].astype(F32)[None, :]
        dt = jnp.exp(ldt_ref[...].astype(F32)[None, :]).astype(BF16).astype(F32)
        mag = jnp.exp(dt * lre)
        ar = mag * jnp.cos(dt * lim)
        ai = mag * jnp.sin(dt * lim)
        den = lre * lre + lim * lim
        nr = ar - 1.0
        cr = 2.0 * (nr * lre + ai * lim) / den
        ci = 2.0 * (ai * lre - nr * lim) / den

        def tiles(x, sign):
            ts = [x[:, 128 * j:128 * (j + 1)] for j in range(3)]
            ts.append(jnp.concatenate([x[:, 384:], sign * x[:, 384:]], axis=1))
            return [jnp.broadcast_to(t, (8, 128)) for t in ts]

        for j, (tr, ti) in enumerate(zip(tiles(ar, 1.0), tiles(ai, -1.0))):
            lam_ref[0, j] = tr
            lam_ref[1, j] = ti
            pr, pi = tr, ti
            n = 1
            while n < SEG:
                pr, pi = _cmul(pr, pi, pr, pi)
                n *= 2
            for lvl in range(3):
                lam_ref[2 + 2 * lvl, j] = jnp.where(sub >= (1 << lvl), pr, 0.0)
                lam_ref[3 + 2 * lvl, j] = jnp.where(sub >= (1 << lvl), pi, 0.0)
                pr, pi = _cmul(pr, pi, pr, pi)
        carry_ref[...] = jnp.zeros(carry_ref.shape, F32)
        dsk = jnp.broadcast_to(dsk_ref[...].astype(F32)[None, :], (128, D))
        dcol_ref[...] = dsk.T
        return cr, ci

    def setup_c(cr, ci):
        for j in range(4):
            cols = slice(128 * j, min(128 * (j + 1), D))
            fr = jnp.broadcast_to(cr[:, cols], (16, cols.stop - cols.start))
            fi = jnp.broadcast_to(ci[:, cols], fr.shape)
            for r in range(0, D, 16):
                c_re = cre_ref[r:r + 16, cols].astype(F32)
                c_im = cim_ref[r:r + 16, cols].astype(F32)
                e_re = c_re * fr - c_im * fi
                e_im = -(c_re * fi + c_im * fr)
                rows = slice(r // 2, r // 2 + 8)
                if j < 3:
                    ccat_ref[rows, 256 * j:256 * j + 128] = _words(e_re)
                    ccat_ref[rows, 256 * j + 128:256 * (j + 1)] = _words(e_im)
                else:
                    ccat_ref[rows, 768:896] = jnp.concatenate([_words(e_re), _words(e_im)], axis=1)

    def by_dim(ref, c, base, e):
        lo = ref[c, pl.ds(base + e, H // 2, stride=DH // 2), :]
        hi = ref[c, pl.ds(base + D // 4 + e, H // 2, stride=DH // 2), :]
        return ((lo & 0xFFFF) | (hi << 16), (lo >> 16) | (hi & np.uint32(0xFFFF0000)))

    def setup_w(m):
        lo, hi = W_COLS[m]
        for n in range(lo, hi, 128):
            n1 = min(n + 128, hi)
            for c in range(4):
                blk = wqkv_ref[128 * c:min(128 * (c + 1), D), n:n1]
                if c == 3:
                    blk = jnp.concatenate([blk, jnp.zeros((DP - D, n1 - n), BF16)], axis=0)
                tmp_ref[c, n // 2:n1 // 2, :] = pltpu.bitcast(blk.T, U32)
        for e in range(DH // 2):
            for c in range(4):
                for i, blk in enumerate(by_dim(tmp_ref, c, m * D // 2, e)):
                    r = m * D // 2 + 8 * (2 * e + i)
                    wt_ref[r:r + 8, 128 * c:128 * (c + 1)] = blk

    def setup_wo():
        for c in range(4):
            cols = 128 if c < 3 else 64
            tmp2_ref[c] = _pad_lanes(pltpu.bitcast(wo_ref[:, 128 * c:128 * c + cols], U32))
        for c in range(4):
            cols = 128 if c < 3 else 64
            wp = jnp.concatenate(
                [blk for e in range(DH // 2) for blk in by_dim(tmp2_ref, c, 0, e)]
                + [jnp.zeros(((DP - D) // 2, 128), U32)], axis=0)
            wot_ref[64 * c:64 * c + cols // 2, :] = pltpu.bitcast(_halves(wp).T[0:cols], U32)

    def transpose_x(b):
        xt_ref[...] = pltpu.bitcast(xa_ref[b].T, U32)

    def ssm_in(tiles):
        for j in tiles:
            if j == 6:
                w = jnp.concatenate([bre_ref[384:448, :], bim_ref[384:448, :]], axis=0)
            else:
                w = (bim_ref if j % 2 else bre_ref)[128 * (j // 2):128 * (j // 2 + 1), :]
            u = lax.dot_general(_halves(xt_ref[...]), w, NT_DIMS, preferred_element_type=F32)
            for jj, uj in ((j, u), (7, pltpu.roll(u, 64, 1))) if j == 6 else ((j, u),):
                for g in range(TB // SEG):
                    s, r = divmod(g, 8)
                    u_ref[s, jj, r * PITCH:r * PITCH + SEG, :] = uj[g * SEG:(g + 1) * SEG]

    def scan(s, pairs=(3, 0, 1, 2)):
        lam = {p: (lam_ref[0, p], lam_ref[1, p]) for p in pairs}

        def step(i, h):
            new = {}
            for p in pairs:
                ur = u_ref[s, 2 * p, pl.ds(i, 8, stride=PITCH), :]
                ui = u_ref[s, 2 * p + 1, pl.ds(i, 8, stride=PITCH), :]
                if h is not None:
                    (ar, ai), (hr, hi) = lam[p], h[p]
                    ur, ui = ar * hr + (ur - ai * hi), ar * hi + (ai * hr + ui)
                new[p] = (ur, ui)
            return new

        h = None
        for i in range(SEG):
            h = step(i, h)
        for p in pairs:
            gr = pltpu.roll(jnp.where(sub == 7, carry_ref[2 * p], h[p][0]), 1, 0)
            gi = pltpu.roll(jnp.where(sub == 7, carry_ref[2 * p + 1], h[p][1]), 1, 0)
            for lvl in range(3):
                mr = lam_ref[2 + 2 * lvl, p]
                mi = lam_ref[3 + 2 * lvl, p]
                sr = pltpu.roll(gr, 1 << lvl, 0)
                si = pltpu.roll(gi, 1 << lvl, 0)
                gr, gi = gr + (mr * sr - mi * si), gi + (mr * si + mi * sr)
            h[p] = (gr, gi)
        for i in range(SEG):
            h = step(i, h)
            for p in pairs:
                for t in range(2 * p, min(2 * p + 2, 7)):
                    h_ref[s, t, pl.ds(i, 8, stride=PITCH), :] = h[p][t % 2]
        for p in pairs:
            carry_ref[2 * p], carry_ref[2 * p + 1] = h[p]

    def ssm_out(b, j, zero=None):
        s, g0 = divmod(j * (128 // SEG), 8)
        h = jnp.concatenate(
            [jnp.concatenate([h_ref[s, t, g * PITCH:g * PITCH + SEG, :]
                              for g in range(g0, g0 + 128 // SEG)], axis=0).astype(BF16)
             for t in range(7)], axis=1)
        if zero is not None:
            h = _halves(pltpu.bitcast(h, U32) | jnp.tile(zero, (8, 7)))
        y_t = lax.dot_general(_halves(ccat_ref[...]), h, NT_DIMS, preferred_element_type=F32)
        return y_t + xa_ref[b, :, 128 * j:128 * (j + 1)].astype(F32) * dcol_ref[...]

    kpad = jnp.zeros((DP - D, 128), BF16)

    def proj(b, m, j, zero=None):
        pad = kpad if zero is None else _halves(jnp.tile(zero, (4, 1)))
        xb = jnp.concatenate([xb_ref[b, :, 128 * j:128 * (j + 1)], pad], axis=0)
        r = jnp.dot(_halves(wt_ref[m * D // 2:(m + 1) * D // 2, :]), xb, preferred_element_type=F32)
        if m == 0:
            q_ref[j] = r
        else:
            dst = k_ref if m == 1 else v_ref
            for d in range(DH):
                dst[j + 1, 8 * d:8 * d + 8, :] = _pack(r[16 * d:16 * d + 8], r[16 * d + 8:16 * d + 16])

    def shifted(prev, cur, w):
        if w == 0:
            return _unpack(cur)
        s = DIL * w
        return _unpack(pltpu.roll(jnp.where(lane >= 128 - s, prev, cur), s, 1))

    def scores(j, first):
        acc = [[None] * WIN for _ in range(2)]
        for w0 in range(0, WIN, 4):
            for d in range(DH):
                qd = [q_ref[j, 16 * d + 8 * hh:16 * d + 8 * hh + 8, :] for hh in range(2)]
                kc = k_ref[j + 1, 8 * d:8 * d + 8, :]
                kp = k_ref[j, 8 * d:8 * d + 8, :]
                for w in range(w0, w0 + 4):
                    ks = shifted(kp, kc, w)
                    for hh in range(2):
                        t = qd[hh] * ks[hh]
                        acc[hh][w] = t if d == 0 else acc[hh][w] + t
        probs = []
        for hh in range(2):
            lg = [a * (DH ** -0.5) for a in acc[hh]]
            if first:
                lg = [lg[0]] + [jnp.where(lane >= DIL * w, lg[w], -1e9) for w in range(1, WIN)]
            mx = lg[0]
            for w in range(1, WIN):
                mx = jnp.maximum(mx, lg[w])
            ex = [jnp.exp(l - mx) for l in lg]
            tot = ex[0]
            for w in range(1, WIN):
                tot = tot + ex[w]
            inv = 1.0 / tot
            probs.append([e * inv for e in ex])
        return probs

    def values(j, probs):
        for d in range(DH):
            vc = v_ref[j + 1, 8 * d:8 * d + 8, :]
            vp = v_ref[j, 8 * d:8 * d + 8, :]
            o = [None, None]
            for w in range(WIN):
                vs = shifted(vp, vc, w)
                for hh in range(2):
                    t = probs[hh][w] * vs[hh]
                    o[hh] = t if w == 0 else o[hh] + t
            ot_ref[j, 8 * d:8 * d + 8, :] = _words(jnp.concatenate(o, axis=0))

    def keep_halo():
        k_ref[0] = k_ref[NT]
        v_ref[0] = v_ref[NT]

    def attn_out(j, zero=None):
        pad = kpad if zero is None else _halves(jnp.tile(zero, (4, 1)))
        o_t = jnp.concatenate([_halves(ot_ref[j]), pad], axis=0)
        return jnp.dot(_halves(wot_ref[...]), o_t, preferred_element_type=F32)

    def finish(b):
        for j in range(NT):
            row = b * TB + 128 * j
            row = row if isinstance(row, int) else pl.multiple_of(row, 128)
            out_ref[pl.ds(row, 128), :] = jnp.concatenate(
                [y_ref[j], attn_out(j)], axis=0).T
        out_copy(b).start()

    def front(b, zero=None):
        transpose_x(b)
        ssm_in((6, 0, 1, 2, 3, 4, 5))
        for j in range(NT):
            for m in (1, 0, 2):
                proj(b, m, j, zero if (j, m) == (0, 1) else None)
            if j < NS:
                scan(j)
            values(j, scores(j, False))
        keep_halo()

    spare_ref[0] = S
    k_ref[0] = jnp.zeros(k_ref.shape[1:], k_ref.dtype)
    v_ref[0] = jnp.zeros(v_ref.shape[1:], v_ref.dtype)
    wait(0)
    transpose_x(0)
    wait(1)
    cr, ci = setup_lambda()
    ssm_in((6, 0, 1, 2,))
    for s in range(NS):
        scan(s, (3, 0,))
    wait(2)
    ssm_in((3, 4, 5,))
    setup_w(1)
    setup_w(0)
    for s in range(NS):
        scan(s, (1,))
    wait(3)
    probs = {}
    setup_w(2)
    proj(0, 1, 0)
    proj(0, 0, 0)
    probs[0] = scores(0, True)
    for s in range(NS):
        scan(s, (2,))
    proj(0, 1, 1)
    proj(0, 0, 1)
    probs[1] = scores(1, False)
    proj(0, 2, 0)
    values(0, probs[0])
    proj(0, 1, 2)
    proj(0, 1, 3)
    wait(4)
    setup_c(cr, ci)
    proj(0, 0, 2)
    probs[2] = scores(2, False)
    proj(0, 0, 3)
    probs[3] = scores(3, False)
    y_ref[0] = ssm_out(0, 0)
    proj(0, 2, 1)
    values(1, probs[1])
    y_ref[1] = ssm_out(0, 1)
    proj(0, 2, 2)
    values(2, probs[2])
    y_ref[2] = ssm_out(0, 2)
    proj(0, 2, 3)
    values(3, probs[3])
    y_ref[3] = ssm_out(0, 3)
    setup_wo()
    keep_halo()

    @pl.loop(1, NB - 1)
    def _(b):
        for cp in x_copies(b + 1):
            cp.start()
        for cp in x_copies(b):
            cp.wait()
        finish(b - 1)
        front(b)
        for j in range(NT):
            y_ref[j] = ssm_out(b, j)

    last = NB - 1
    for cp in x_copies(last):
        cp.wait()
    spare = pl.multiple_of(spare_ref[0], 8)

    def after_start():
        out_ref[S:S + 8, 0:128] = jnp.zeros((8, 128), F32)
        return pltpu.bitcast(out_ref[pl.ds(spare, 8), 0:128], U32)

    finish(last - 1)
    front(last, after_start())
    stores = [out_copy(b) for b in range(last)]
    gates = [None] * 3

    def emit(j, lo, hi, t):
        out_ref[last * TB + 128 * j:last * TB + 128 * (j + 1), lo:hi] = t.T
        stores.append(tail_copy(j, lo, hi))
        stores[-1].start()

    for j in range(NT):
        y_t = ssm_out(last, j)
        emit(j, 0, 384, y_t[0:384])
        gates.append(after_start())
        rest = jnp.concatenate([y_t[384:D], attn_out(j, gates[-3] if j > 1 else None)], axis=0)
        cuts = (384, 768, 896) if j == NT - 1 else (384, 896)
        for lo, hi in zip(cuts, cuts[1:]):
            emit(j, lo, hi, rest[lo - 384:hi - 384])
        gates.append(after_start())
    for cp in stores:
        cp.wait()


@jax.jit
def pallas_concat_heads__ssm_conv_s5__sliding_local_dilated__prompt_kernel(
    A_x, A_Lambda_re, A_Lambda_im, A_B_re, A_B_im, A_C_re, A_C_im, A_log_dt, A_Dskip,
    B_x, B_wqkv, B_wo,
):
    xa_t = jnp.swapaxes(A_x[0], 0, 1)
    xb_t = jnp.swapaxes(B_x[0], 0, 1)
    hbm = pl.BlockSpec(memory_space=pltpu.HBM)
    vm = pltpu.VMEM
    out = pl.pallas_call(
        _kernel,
        in_specs=[hbm] * 12,
        out_specs=hbm,
        out_shape=jax.ShapeDtypeStruct((S, 2 * D), F32),
        scratch_shapes=[
            vm((NB, D, TB), BF16), vm((NB, D, TB), BF16),
            vm((D,), BF16), vm((D,), BF16), vm((D,), BF16), vm((D,), BF16),
            vm((D, D), BF16), vm((D, D), BF16), vm((D, D), BF16), vm((D, D), BF16),
            vm((D, 3 * D), BF16), vm((D, D), BF16),
            vm((8, 4, 8, 128), F32),
            vm((8, 8, 128), F32),
            vm((D // 2, 2 * D), U32),
            vm((3 * D // 2, DP), U32),
            vm((D // 2, DP), U32),
            vm((D, 128), F32),
            vm((4, 3 * D // 2, 128), U32),
            vm((4, D // 2, 128), U32),
            vm((TB // 2, D), U32),
            vm((NS, 8, 8 * PITCH, 128), F32),
            vm((NS, 7, 8 * PITCH, 128), F32),
            vm((NT, D, 128), F32),
            vm((NT + 1, D // 2, 128), U32),
            vm((NT + 1, D // 2, 128), U32),
            vm((NT, D // 2, 128), U32),
            vm((NT, D, 128), F32),
            vm((S + 8, 2 * D), F32),
            pltpu.SMEM((1,), jnp.int32),
            pltpu.SemaphoreType.DMA((4 + NB,)),
            pltpu.SemaphoreType.DMA(()),
        ],
        compiler_params=pltpu.CompilerParams(vmem_limit_bytes=100 * 1024 * 1024),
    )(xa_t, xb_t, A_Lambda_re, A_Lambda_im, A_log_dt, A_Dskip,
      A_B_re, A_B_im, A_C_re, A_C_im, B_wqkv, B_wo)
    return out[None]
```

```python
import jax
import jax.numpy as jnp
import numpy as np
from jax import lax
import jax.experimental.pallas as pl
import jax.experimental.pallas.tpu as pltpu

S = 2048
D = 448
DP = 512
H = 16
DH = D // H
WIN = 8
DIL = 2
TB = 512
NB = S // TB
NT = TB // 128
SB = 256
NS = TB // SB
SEG = SB // 8
PITCH = SEG + 1
Q, K, V = range(3)
W_COLS = ((0, 384), (384, 896), (896, 3 * D))
F32 = jnp.float32
BF16 = jnp.bfloat16
U32 = jnp.uint32
NT_DIMS = (((1,), (1,)), ((), ()))


def _cmul(ar, ai, br, bi):
    return ar * br - ai * bi, ar * bi + ai * br


def _words(x):
    return pltpu.bitcast(x.astype(BF16), U32)


def _halves(w):
    return pltpu.bitcast(w, BF16)


def _kernel(xa_hbm, xb_hbm, lre_hbm, lim_hbm, ldt_hbm, dsk_hbm,
            bre_hbm, bim_hbm, cre_hbm, cim_hbm, wqkv_hbm, wo_hbm,
            out_hbm,
            xa_ref, xb_ref, lre_ref, lim_ref, ldt_ref, dsk_ref,
            bre_ref, bim_ref, cre_ref, cim_ref, wqkv_ref, wo_ref,
            lam_ref, carry_ref, ccat_ref, wt_ref, wot_ref, dcol_ref, tmp_ref, tmp2_ref,
            xt_ref, u_ref, h_ref, q_ref, k_ref, v_ref, ot_ref, y_ref, out_ref, spare_ref,
            isem, osem):
    def tokens(b):
        return pl.ds(b * TB if isinstance(b, int) else pl.multiple_of(b * TB, TB), TB)

    def rows_of(hbm, ref, lo, hi):
        return hbm.at[pl.ds(lo, hi - lo)], ref.at[pl.ds(lo, hi - lo)]

    def w_cols(m):
        cols = pl.ds(W_COLS[m][0], W_COLS[m][1] - W_COLS[m][0])
        return wqkv_hbm.at[:, cols], wqkv_ref.at[:, cols]

    groups = [
        [(xa_hbm.at[:, tokens(0)], xa_ref.at[0]), rows_of(bre_hbm, bre_ref, 0, 128)],
        [(lre_hbm, lre_ref), (lim_hbm, lim_ref), (ldt_hbm, ldt_ref), (dsk_hbm, dsk_ref),
         rows_of(bre_hbm, bre_ref, 384, D), rows_of(bim_hbm, bim_ref, 384, D),
         rows_of(bim_hbm, bim_ref, 0, 256), rows_of(bre_hbm, bre_ref, 128, 256)],
        [rows_of(bre_hbm, bre_ref, 256, 384), rows_of(bim_hbm, bim_ref, 256, 384), w_cols(K)],
        [w_cols(Q), (xb_hbm.at[:, tokens(0)], xb_ref.at[0])],
        [w_cols(V)],
        [(cre_hbm, cre_ref), (cim_hbm, cim_ref), (wo_hbm, wo_ref)],
    ]
    groups = [[pltpu.make_async_copy(src, dst, isem.at[g]) for src, dst in group]
              for g, group in enumerate(groups)]

    def x_copies(b):
        return [pltpu.make_async_copy(hbm.at[:, tokens(b)], ref.at[b],
                                      isem.at[len(groups) - 1 + b])
                for hbm, ref in ((xa_hbm, xa_ref), (xb_hbm, xb_ref))]

    def out_copy(b):
        return pltpu.make_async_copy(out_ref.at[tokens(b)], out_hbm.at[tokens(b)], osem)

    def start(copies):
        for cp in copies:
            cp.start()

    def wait(copies):
        for cp in copies:
            cp.wait()

    sub = lax.broadcasted_iota(jnp.int32, (8, 128), 0)
    lane = lax.broadcasted_iota(jnp.int32, (8, 128), 1)

    def setup_lambda():
        lre = lre_ref[...].astype(F32)[None, :]
        lim = lim_ref[...].astype(F32)[None, :]
        dt = jnp.exp(ldt_ref[...].astype(F32)[None, :]).astype(BF16).astype(F32)
        mag = jnp.exp(dt * lre)
        ar = mag * jnp.cos(dt * lim)
        ai = mag * jnp.sin(dt * lim)
        den = lre * lre + lim * lim
        fr = 2.0 * ((ar - 1.0) * lre + ai * lim) / den
        fi = 2.0 * (ai * lre - (ar - 1.0) * lim) / den

        def tiles(x, sign):
            ts = [x[:, 128 * j:128 * (j + 1)] for j in range(3)]
            ts.append(jnp.concatenate([x[:, 384:], sign * x[:, 384:]], axis=1))
            return [jnp.broadcast_to(t, (8, 128)) for t in ts]

        for p, (pr, pi) in enumerate(zip(tiles(ar, 1.0), tiles(ai, -1.0))):
            lam_ref[0, p] = pr
            lam_ref[1, p] = pi
            for _ in range(SEG.bit_length() - 1):
                pr, pi = _cmul(pr, pi, pr, pi)
            for lvl in range(3):
                lam_ref[2 + 2 * lvl, p] = jnp.where(sub >= (1 << lvl), pr, 0.0)
                lam_ref[3 + 2 * lvl, p] = jnp.where(sub >= (1 << lvl), pi, 0.0)
                pr, pi = _cmul(pr, pi, pr, pi)
        carry_ref[...] = jnp.zeros(carry_ref.shape, F32)
        dcol_ref[...] = jnp.broadcast_to(dsk_ref[...].astype(F32)[None, :], (128, D)).T
        return fr, fi

    def setup_c(fr, fi):
        for j in range(4):
            cols = slice(128 * j, min(128 * (j + 1), D))
            gr = jnp.broadcast_to(fr[:, cols], (16, cols.stop - cols.start))
            gi = jnp.broadcast_to(fi[:, cols], gr.shape)
            for r in range(0, D, 16):
                e_re, e_im = _cmul(cre_ref[r:r + 16, cols].astype(F32),
                                   cim_ref[r:r + 16, cols].astype(F32), gr, gi)
                rows = slice(r // 2, r // 2 + 8)
                if j < 3:
                    ccat_ref[rows, 256 * j:256 * j + 128] = _words(e_re)
                    ccat_ref[rows, 256 * j + 128:256 * (j + 1)] = _words(-e_im)
                else:
                    ccat_ref[rows, 768:896] = jnp.concatenate(
                        [_words(e_re), _words(-e_im)], axis=1)

    def by_dim(ref, c, base, e):
        lo = ref[c, pl.ds(base + e, H // 2, stride=DH), :]
        hi = ref[c, pl.ds(base + DH // 2 + e, H // 2, stride=DH), :]
        return (lo & 0xFFFF) | (hi << 16), (lo >> 16) | (hi & np.uint32(0xFFFF0000))

    def setup_w(m):
        lo, hi = W_COLS[m]
        for n in range(lo, hi, 128):
            n1 = min(n + 128, hi)
            for c in range(4):
                blk = wqkv_ref[128 * c:min(128 * (c + 1), D), n:n1]
                if c == 3:
                    blk = jnp.concatenate([blk, jnp.zeros((DP - D, n1 - n), BF16)], axis=0)
                tmp_ref[c, n // 2:n1 // 2, :] = pltpu.bitcast(blk.T, U32)
        for e in range(DH // 2):
            for c in range(4):
                for i, blk in enumerate(by_dim(tmp_ref, c, m * D // 2, e)):
                    r = m * D // 2 + 8 * (2 * e + i)
                    wt_ref[r:r + 8, 128 * c:128 * (c + 1)] = blk

    def setup_wo():
        for c in range(4):
            blk = pltpu.bitcast(wo_ref[:, 128 * c:min(128 * (c + 1), D)], U32)
            if c == 3:
                blk = jnp.concatenate([blk, jnp.zeros((D // 2, DP - D), U32)], axis=1)
            tmp2_ref[c] = blk
        for c in range(4):
            cols = min(128, D - 128 * c)
            wp = jnp.concatenate(
                [blk for e in range(DH // 2) for blk in by_dim(tmp2_ref, c, 0, e)]
                + [jnp.zeros(((DP - D) // 2, 128), U32)], axis=0)
            wot_ref[64 * c:64 * c + cols // 2, :] = pltpu.bitcast(_halves(wp).T[0:cols], U32)

    def transpose_x(b):
        xt_ref[...] = pltpu.bitcast(xa_ref[b].T, U32)

    def ssm_in(tiles):
        for j in tiles:
            if j == 6:
                w = jnp.concatenate([bre_ref[384:D, :], bim_ref[384:D, :]], axis=0)
            else:
                w = (bim_ref if j % 2 else bre_ref)[128 * (j // 2):128 * (j // 2 + 1), :]
            u = lax.dot_general(_halves(xt_ref[...]), w, NT_DIMS, preferred_element_type=F32)
            for t, ut in ((6, u), (7, pltpu.roll(u, 64, 1))) if j == 6 else ((j, u),):
                for g in range(TB // SEG):
                    s, r = divmod(g, 8)
                    u_ref[s, t, r * PITCH:r * PITCH + SEG, :] = ut[g * SEG:(g + 1) * SEG]

    def scan(s, pairs):
        lam = {p: (lam_ref[0, p], lam_ref[1, p]) for p in pairs}

        def step(i, h):
            new = {}
            for p in pairs:
                ur = u_ref[s, 2 * p, pl.ds(i, 8, stride=PITCH), :]
                ui = u_ref[s, 2 * p + 1, pl.ds(i, 8, stride=PITCH), :]
                if h is not None:
                    (ar, ai), (hr, hi) = lam[p], h[p]
                    ur, ui = ar * hr + (ur - ai * hi), ar * hi + (ai * hr + ui)
                new[p] = (ur, ui)
            return new

        h = None
        for i in range(SEG):
            h = step(i, h)
        for p in pairs:
            gr = pltpu.roll(jnp.where(sub == 7, carry_ref[2 * p], h[p][0]), 1, 0)
            gi = pltpu.roll(jnp.where(sub == 7, carry_ref[2 * p + 1], h[p][1]), 1, 0)
            for lvl in range(3):
                tr, ti = _cmul(lam_ref[2 + 2 * lvl, p], lam_ref[3 + 2 * lvl, p],
                               pltpu.roll(gr, 1 << lvl, 0), pltpu.roll(gi, 1 << lvl, 0))
                gr, gi = gr + tr, gi + ti
            h[p] = (gr, gi)
        for i in range(SEG):
            h = step(i, h)
            for p in pairs:
                for t in range(2 * p, min(2 * p + 2, 7)):
                    h_ref[s, t, pl.ds(i, 8, stride=PITCH), :] = h[p][t % 2]
        for p in pairs:
            carry_ref[2 * p], carry_ref[2 * p + 1] = h[p]

    def scan_block(pairs):
        for s in range(NS):
            scan(s, pairs)

    def ssm_out(b, j, lo=0, hi=D, zero=None):
        s, g0 = divmod(j * (128 // SEG), 8)
        h = jnp.concatenate(
            [jnp.concatenate([h_ref[s, t, g * PITCH:g * PITCH + SEG, :]
                              for g in range(g0, g0 + 128 // SEG)], axis=0).astype(BF16)
             for t in range(7)], axis=1)
        if zero is not None:
            zero = jnp.concatenate([jnp.concatenate([zero] * 8, axis=0)] * 7, axis=1)
            h = _halves(pltpu.bitcast(h, U32) | zero)
        y_t = lax.dot_general(_halves(ccat_ref[lo // 2:hi // 2, :]), h, NT_DIMS,
                              preferred_element_type=F32)
        return y_t + xa_ref[b, lo:hi, 128 * j:128 * (j + 1)].astype(F32) * dcol_ref[lo:hi, :]

    def padded(x, zero):
        pad = (jnp.zeros((DP - D, 128), BF16) if zero is None
               else _halves(jnp.concatenate([zero] * 4, axis=0)))
        return jnp.concatenate([x, pad], axis=0)

    def proj(b, m, j, zero=None):
        r = jnp.dot(_halves(wt_ref[m * D // 2:(m + 1) * D // 2, :]),
                    padded(xb_ref[b, :, 128 * j:128 * (j + 1)], zero),
                    preferred_element_type=F32)
        if m == Q:
            q_ref[j] = r
        else:
            (k_ref if m == K else v_ref)[j + 1] = _words(r)

    def shifted(prev, cur, w):
        if w:
            cur = pltpu.roll(jnp.where(lane >= 128 - DIL * w, prev, cur), DIL * w, 1)
        cur = _halves(cur).astype(F32)
        return cur[0:8], cur[8:16]

    def scores(j, first=False):
        acc = [[None] * WIN for _ in range(2)]
        for w0 in range(0, WIN, 4):
            for d in range(DH):
                qd = [q_ref[j, 16 * d + 8 * hh:16 * d + 8 * hh + 8, :] for hh in range(2)]
                cur, prev = k_ref[j + 1, 8 * d:8 * d + 8, :], k_ref[j, 8 * d:8 * d + 8, :]
                for w in range(w0, w0 + 4):
                    ks = shifted(prev, cur, w)
                    for hh in range(2):
                        t = qd[hh] * ks[hh]
                        acc[hh][w] = t if d == 0 else acc[hh][w] + t
        probs = []
        for hh in range(2):
            lg = [a * (DH ** -0.5) for a in acc[hh]]
            if first:
                lg = [lg[0]] + [jnp.where(lane >= DIL * w, lg[w], -1e9) for w in range(1, WIN)]
            mx = lg[0]
            for w in range(1, WIN):
                mx = jnp.maximum(mx, lg[w])
            ex = [jnp.exp(t - mx) for t in lg]
            tot = ex[0]
            for w in range(1, WIN):
                tot = tot + ex[w]
            inv = 1.0 / tot
            probs.append([e * inv for e in ex])
        return probs

    def values(j, probs):
        for d in range(DH):
            cur, prev = v_ref[j + 1, 8 * d:8 * d + 8, :], v_ref[j, 8 * d:8 * d + 8, :]
            o = [None, None]
            for w in range(WIN):
                vs = shifted(prev, cur, w)
                for hh in range(2):
                    t = probs[hh][w] * vs[hh]
                    o[hh] = t if w == 0 else o[hh] + t
            ot_ref[j, 8 * d:8 * d + 8, :] = _words(jnp.concatenate(o, axis=0))

    def keep_history():
        k_ref[0] = k_ref[NT]
        v_ref[0] = v_ref[NT]

    def attn_out(j, zero=None):
        return jnp.dot(_halves(wot_ref[...]), padded(_halves(ot_ref[j]), zero),
                       preferred_element_type=F32)

    def front(b, zero=None):
        transpose_x(b)
        ssm_in((6, 0, 1, 2, 3, 4, 5))
        for j in range(NT):
            proj(b, K, j, zero if j == 0 else None)
            proj(b, Q, j)
            proj(b, V, j)
            if j < NS:
                scan(j, (3, 0, 1, 2))
            values(j, scores(j))
        keep_history()

    def finish(b):
        for j in range(NT):
            row = b * TB + 128 * j
            row = row if isinstance(row, int) else pl.multiple_of(row, 128)
            out_ref[pl.ds(row, 128), :] = jnp.concatenate([y_ref[j], attn_out(j)], axis=0).T
        out_copy(b).start()

    for group in groups:
        start(group)
    start(x_copies(1))
    spare_ref[0] = S
    k_ref[0] = jnp.zeros(k_ref.shape[1:], U32)
    wait(groups[0])
    transpose_x(0)
    ssm_in((0,))
    wait(groups[1])
    fr, fi = setup_lambda()
    ssm_in((6, 1, 2, 3))
    scan_block((3, 0))
    wait(groups[2])
    ssm_in((4, 5))
    scan_block((1,))
    setup_w(K)
    wait(groups[3])
    setup_w(Q)
    proj(0, K, 0)
    proj(0, K, 1)
    scan_block((2,))
    wait(groups[4])
    setup_w(V)
    proj(0, Q, 0)
    p0 = scores(0, first=True)
    proj(0, Q, 1)
    p1 = scores(1)
    proj(0, V, 0)
    v_ref[0] = jnp.broadcast_to(v_ref[1][:, 0:1], v_ref.shape[1:])
    values(0, p0)
    proj(0, K, 2)
    proj(0, K, 3)
    wait(groups[5])
    setup_c(fr, fi)
    proj(0, Q, 2)
    p2 = scores(2)
    proj(0, Q, 3)
    p3 = scores(3)
    y_ref[0] = ssm_out(0, 0)
    for j, p in ((1, p1), (2, p2), (3, p3)):
        proj(0, V, j)
        values(j, p)
        y_ref[j] = ssm_out(0, j)
    keep_history()
    setup_wo()

    @pl.loop(1, NB - 1)
    def _(b):
        start(x_copies(b + 1))
        wait(x_copies(b))
        finish(b - 1)
        front(b)
        for j in range(NT):
            y_ref[j] = ssm_out(b, j)

    last = NB - 1
    wait(x_copies(last))
    spare = pl.multiple_of(spare_ref[0], 8)
    stores = [out_copy(b) for b in range(last)]

    def zero_after_start():
        out_ref[S:S + 8, 0:128] = jnp.zeros((8, 128), F32)
        return pltpu.bitcast(out_ref[pl.ds(spare, 8), 0:128], U32)

    def emit(j, lo, hi, t):
        rows, cols = pl.ds(last * TB + 128 * j, 128), pl.ds(lo, hi - lo)
        out_ref[rows, cols] = t.T
        stores.append(pltpu.make_async_copy(out_ref.at[rows, cols], out_hbm.at[rows, cols], osem))
        stores[-1].start()
        return zero_after_start()

    finish(last - 1)
    front(last, zero_after_start())
    sent = [None, None]
    for j in range(NT - 1):
        y_t = ssm_out(last, j)
        sent.append(emit(j, 0, 384, y_t[0:384]))
        ob_t = attn_out(j, sent[-3] if j > 1 else None)
        sent.append(emit(j, 384, 896, jnp.concatenate([y_t[384:D], ob_t], axis=0)))
    j = NT - 1
    ob_t = attn_out(j, sent[-2])
    zero = emit(j, 512, 896, ob_t[64:D])
    emit(j, 0, 384, ssm_out(last, j, 0, 384))
    emit(j, 384, 512, jnp.concatenate([ssm_out(last, j, 384, D, zero), ob_t[0:64]], axis=0))
    wait(stores)


@jax.jit
def pallas_concat_heads__ssm_conv_s5__sliding_local_dilated__prompt_kernel(
    A_x: jax.Array,
    A_Lambda_re: jax.Array,
    A_Lambda_im: jax.Array,
    A_B_re: jax.Array,
    A_B_im: jax.Array,
    A_C_re: jax.Array,
    A_C_im: jax.Array,
    A_log_dt: jax.Array,
    A_Dskip: jax.Array,
    B_x: jax.Array,
    B_wqkv: jax.Array,
    B_wo: jax.Array,
):
    hbm = pl.BlockSpec(memory_space=pltpu.HBM)
    vm = pltpu.VMEM
    out = pl.pallas_call(
        _kernel,
        in_specs=[hbm] * 12,
        out_specs=hbm,
        out_shape=jax.ShapeDtypeStruct((S, 2 * D), F32),
        scratch_shapes=[
            vm((NB, D, TB), BF16), vm((NB, D, TB), BF16),
            vm((D,), BF16), vm((D,), BF16), vm((D,), BF16), vm((D,), BF16),
            vm((D, D), BF16), vm((D, D), BF16), vm((D, D), BF16), vm((D, D), BF16),
            vm((D, 3 * D), BF16), vm((D, D), BF16),
            vm((8, 4, 8, 128), F32),
            vm((8, 8, 128), F32),
            vm((D // 2, 2 * D), U32),
            vm((3 * D // 2, DP), U32),
            vm((D // 2, DP), U32),
            vm((D, 128), F32),
            vm((4, 3 * D // 2, 128), U32),
            vm((4, D // 2, 128), U32),
            vm((TB // 2, D), U32),
            vm((NS, 8, 8 * PITCH, 128), F32),
            vm((NS, 7, 8 * PITCH, 128), F32),
            vm((NT, D, 128), F32),
            vm((NT + 1, D // 2, 128), U32),
            vm((NT + 1, D // 2, 128), U32),
            vm((NT, D // 2, 128), U32),
            vm((NT, D, 128), F32),
            vm((S + 8, 2 * D), F32),
            pltpu.SMEM((1,), jnp.int32),
            pltpu.SemaphoreType.DMA((5 + NB,)),
            pltpu.SemaphoreType.DMA(()),
        ],
        compiler_params=pltpu.CompilerParams(vmem_limit_bytes=64 * 1024 * 1024),
    )(A_x.reshape(S, D).T, B_x.reshape(S, D).T, A_Lambda_re, A_Lambda_im, A_log_dt, A_Dskip,
      A_B_re, A_B_im, A_C_re, A_C_im, B_wqkv, B_wo)
    return out.reshape(1, S, 2 * D)
```

```python
import jax
import jax.numpy as jnp
import numpy as np
from jax import lax
import jax.experimental.pallas as pl
import jax.experimental.pallas.tpu as pltpu

S = 2048
D = 448
DP = 512
H = 16
DH = D // H
WIN = 8
DIL = 2
TB = 512
NB = S // TB
NT = TB // 128
SB = 256
NS = TB // SB
SEG = SB // 8
PITCH = SEG + 1
Q, K, V = range(3)
W_COLS = ((0, 384), (384, 896), (896, 3 * D))
F32 = jnp.float32
BF16 = jnp.bfloat16
U32 = jnp.uint32
NT_DIMS = (((1,), (1,)), ((), ()))


def _cmul(ar, ai, br, bi):
    return ar * br - ai * bi, ar * bi + ai * br


def _words(x):
    return pltpu.bitcast(x.astype(BF16), U32)


def _halves(w):
    return pltpu.bitcast(w, BF16)


def _kernel(xa_hbm, xb_hbm, lre_hbm, lim_hbm, ldt_hbm, dsk_hbm,
            bre_hbm, bim_hbm, cre_hbm, cim_hbm, wqkv_hbm, wo_hbm,
            out_hbm,
            xa_ref, xb_ref, lre_ref, lim_ref, ldt_ref, dsk_ref,
            bre_ref, bim_ref, cre_ref, cim_ref, wqkv_ref, wo_ref,
            lam_ref, carry_ref, ccat_ref, wt_ref, wot_ref, dcol_ref, tmp_ref, tmp2_ref,
            xt_ref, u_ref, h_ref, q_ref, k_ref, v_ref, ot_ref, y_ref, out_ref, spare_ref,
            isem, osem):
    def tokens(b):
        return pl.ds(b * TB if isinstance(b, int) else pl.multiple_of(b * TB, TB), TB)

    def rows_of(hbm, ref, lo, hi):
        return hbm.at[pl.ds(lo, hi - lo)], ref.at[pl.ds(lo, hi - lo)]

    def w_cols(m):
        cols = pl.ds(W_COLS[m][0], W_COLS[m][1] - W_COLS[m][0])
        return wqkv_hbm.at[:, cols], wqkv_ref.at[:, cols]

    groups = [
        [(xa_hbm.at[:, tokens(0)], xa_ref.at[0]), rows_of(bre_hbm, bre_ref, 0, 128)],
        [(lre_hbm, lre_ref), (lim_hbm, lim_ref), (ldt_hbm, ldt_ref), (dsk_hbm, dsk_ref),
         rows_of(bre_hbm, bre_ref, 384, D), rows_of(bim_hbm, bim_ref, 384, D),
         rows_of(bim_hbm, bim_ref, 0, 256), rows_of(bre_hbm, bre_ref, 128, 256)],
        [rows_of(bre_hbm, bre_ref, 256, 384), rows_of(bim_hbm, bim_ref, 256, 384), w_cols(K)],
        [w_cols(Q), (xb_hbm.at[:, tokens(0)], xb_ref.at[0])],
        [w_cols(V)],
        [(cre_hbm, cre_ref), (cim_hbm, cim_ref), (wo_hbm, wo_ref)],
    ]
    groups = [[pltpu.make_async_copy(src, dst, isem.at[g]) for src, dst in group]
              for g, group in enumerate(groups)]

    def x_copies(b):
        return [pltpu.make_async_copy(hbm.at[:, tokens(b)], ref.at[b],
                                      isem.at[len(groups) - 1 + b])
                for hbm, ref in ((xa_hbm, xa_ref), (xb_hbm, xb_ref))]

    def out_copy(b):
        return pltpu.make_async_copy(out_ref.at[tokens(b)], out_hbm.at[tokens(b)], osem)

    def start(copies):
        for cp in copies:
            cp.start()

    def wait(copies):
        for cp in copies:
            cp.wait()

    sub = lax.broadcasted_iota(jnp.int32, (8, 128), 0)
    lane = lax.broadcasted_iota(jnp.int32, (8, 128), 1)

    def setup_lambda():
        lre = lre_ref[...].astype(F32)[None, :]
        lim = lim_ref[...].astype(F32)[None, :]
        dt = jnp.exp(ldt_ref[...].astype(F32)[None, :]).astype(BF16).astype(F32)
        mag = jnp.exp(dt * lre)
        ar = mag * jnp.cos(dt * lim)
        ai = mag * jnp.sin(dt * lim)
        big = jnp.maximum(jnp.abs(lre), jnp.abs(lim))
        nre, nim = lre / big, lim / big
        den = nre * lre + nim * lim
        fr = 2.0 * ((ar - 1.0) * nre + ai * nim) / den
        fi = 2.0 * (ai * nre - (ar - 1.0) * nim) / den

        def tiles(x, sign):
            ts = [x[:, 128 * j:128 * (j + 1)] for j in range(3)]
            ts.append(jnp.concatenate([x[:, 384:], sign * x[:, 384:]], axis=1))
            return [jnp.broadcast_to(t, (8, 128)) for t in ts]

        for p, (pr, pi) in enumerate(zip(tiles(ar, 1.0), tiles(ai, -1.0))):
            lam_ref[0, p] = pr
            lam_ref[1, p] = pi
            for _ in range(SEG.bit_length() - 1):
                pr, pi = _cmul(pr, pi, pr, pi)
            for lvl in range(3):
                lam_ref[2 + 2 * lvl, p] = jnp.where(sub >= (1 << lvl), pr, 0.0)
                lam_ref[3 + 2 * lvl, p] = jnp.where(sub >= (1 << lvl), pi, 0.0)
                pr, pi = _cmul(pr, pi, pr, pi)
        carry_ref[...] = jnp.zeros(carry_ref.shape, F32)
        dcol_ref[...] = jnp.broadcast_to(dsk_ref[...].astype(F32)[None, :], (128, D)).T
        return fr, fi

    def setup_c(fr, fi):
        for j in range(4):
            cols = slice(128 * j, min(128 * (j + 1), D))
            gr = jnp.broadcast_to(fr[:, cols], (16, cols.stop - cols.start))
            gi = jnp.broadcast_to(fi[:, cols], gr.shape)
            for r in range(0, D, 16):
                e_re, e_im = _cmul(cre_ref[r:r + 16, cols].astype(F32),
                                   cim_ref[r:r + 16, cols].astype(F32), gr, gi)
                rows = slice(r // 2, r // 2 + 8)
                if j < 3:
                    ccat_ref[rows, 256 * j:256 * j + 128] = _words(e_re)
                    ccat_ref[rows, 256 * j + 128:256 * (j + 1)] = _words(-e_im)
                else:
                    ccat_ref[rows, 768:896] = jnp.concatenate(
                        [_words(e_re), _words(-e_im)], axis=1)

    def by_dim(ref, c, base, e):
        lo = ref[c, pl.ds(base + e, H // 2, stride=DH), :]
        hi = ref[c, pl.ds(base + DH // 2 + e, H // 2, stride=DH), :]
        return (lo & 0xFFFF) | (hi << 16), (lo >> 16) | (hi & np.uint32(0xFFFF0000))

    def setup_w(m):
        lo, hi = W_COLS[m]
        for n in range(lo, hi, 128):
            n1 = min(n + 128, hi)
            for c in range(4):
                blk = wqkv_ref[128 * c:min(128 * (c + 1), D), n:n1]
                if c == 3:
                    blk = jnp.concatenate([blk, jnp.zeros((DP - D, n1 - n), BF16)], axis=0)
                tmp_ref[c, n // 2:n1 // 2, :] = pltpu.bitcast(blk.T, U32)
        for e in range(DH // 2):
            for c in range(4):
                for i, blk in enumerate(by_dim(tmp_ref, c, m * D // 2, e)):
                    r = m * D // 2 + 8 * (2 * e + i)
                    wt_ref[r:r + 8, 128 * c:128 * (c + 1)] = blk

    def setup_wo():
        for c in range(4):
            blk = pltpu.bitcast(wo_ref[:, 128 * c:min(128 * (c + 1), D)], U32)
            if c == 3:
                blk = jnp.concatenate([blk, jnp.zeros((D // 2, DP - D), U32)], axis=1)
            tmp2_ref[c] = blk
        for c in range(4):
            cols = min(128, D - 128 * c)
            wp = jnp.concatenate(
                [blk for e in range(DH // 2) for blk in by_dim(tmp2_ref, c, 0, e)]
                + [jnp.zeros(((DP - D) // 2, 128), U32)], axis=0)
            wot_ref[64 * c:64 * c + cols // 2, :] = pltpu.bitcast(_halves(wp).T[0:cols], U32)

    def transpose_x(b):
        xt_ref[...] = pltpu.bitcast(xa_ref[b].T, U32)

    def ssm_in(tiles):
        for j in tiles:
            if j == 6:
                w = jnp.concatenate([bre_ref[384:D, :], bim_ref[384:D, :]], axis=0)
            else:
                w = (bim_ref if j % 2 else bre_ref)[128 * (j // 2):128 * (j // 2 + 1), :]
            u = lax.dot_general(_halves(xt_ref[...]), w, NT_DIMS, preferred_element_type=F32)
            for t, ut in ((6, u), (7, pltpu.roll(u, 64, 1))) if j == 6 else ((j, u),):
                for g in range(TB // SEG):
                    s, r = divmod(g, 8)
                    u_ref[s, t, r * PITCH:r * PITCH + SEG, :] = ut[g * SEG:(g + 1) * SEG]

    def scan(s, pairs):
        lam = {p: (lam_ref[0, p], lam_ref[1, p]) for p in pairs}

        def step(i, h):
            new = {}
            for p in pairs:
                ur = u_ref[s, 2 * p, pl.ds(i, 8, stride=PITCH), :]
                ui = u_ref[s, 2 * p + 1, pl.ds(i, 8, stride=PITCH), :]
                if h is not None:
                    (ar, ai), (hr, hi) = lam[p], h[p]
                    ur, ui = ar * hr + (ur - ai * hi), ar * hi + (ai * hr + ui)
                new[p] = (ur, ui)
            return new

        h = None
        for i in range(SEG):
            h = step(i, h)
        for p in pairs:
            gr = pltpu.roll(jnp.where(sub == 7, carry_ref[2 * p], h[p][0]), 1, 0)
            gi = pltpu.roll(jnp.where(sub == 7, carry_ref[2 * p + 1], h[p][1]), 1, 0)
            for lvl in range(3):
                tr, ti = _cmul(lam_ref[2 + 2 * lvl, p], lam_ref[3 + 2 * lvl, p],
                               pltpu.roll(gr, 1 << lvl, 0), pltpu.roll(gi, 1 << lvl, 0))
                gr, gi = gr + tr, gi + ti
            h[p] = (gr, gi)
        for i in range(SEG):
            h = step(i, h)
            for p in pairs:
                for t in range(2 * p, min(2 * p + 2, 7)):
                    h_ref[s, t, pl.ds(i, 8, stride=PITCH), :] = h[p][t % 2]
        for p in pairs:
            carry_ref[2 * p], carry_ref[2 * p + 1] = h[p]

    def scan_block(pairs):
        for s in range(NS):
            scan(s, pairs)

    def ssm_out(b, j, lo=0, hi=D, zero=None):
        s, g0 = divmod(j * (128 // SEG), 8)
        h = jnp.concatenate(
            [jnp.concatenate([h_ref[s, t, g * PITCH:g * PITCH + SEG, :]
                              for g in range(g0, g0 + 128 // SEG)], axis=0).astype(BF16)
             for t in range(7)], axis=1)
        if zero is not None:
            zero = jnp.concatenate([jnp.concatenate([zero] * 8, axis=0)] * 7, axis=1)
            h = _halves(pltpu.bitcast(h, U32) | zero)
        y_t = lax.dot_general(_halves(ccat_ref[lo // 2:hi // 2, :]), h, NT_DIMS,
                              preferred_element_type=F32)
        return y_t + xa_ref[b, lo:hi, 128 * j:128 * (j + 1)].astype(F32) * dcol_ref[lo:hi, :]

    def padded(x, zero):
        pad = (jnp.zeros((DP - D, 128), BF16) if zero is None
               else _halves(jnp.concatenate([zero] * 4, axis=0)))
        return jnp.concatenate([x, pad], axis=0)

    def proj(b, m, j, zero=None):
        r = jnp.dot(_halves(wt_ref[m * D // 2:(m + 1) * D // 2, :]),
                    padded(xb_ref[b, :, 128 * j:128 * (j + 1)], zero),
                    preferred_element_type=F32)
        if m == Q:
            q_ref[j] = r
        else:
            (k_ref if m == K else v_ref)[j + 1] = _words(r)

    def shifted(prev, cur, w):
        if w:
            cur = pltpu.roll(jnp.where(lane >= 128 - DIL * w, prev, cur), DIL * w, 1)
        cur = _halves(cur).astype(F32)
        return cur[0:8], cur[8:16]

    def scores(j, first=False):
        acc = [[None] * WIN for _ in range(2)]
        for w0 in range(0, WIN, 4):
            for d in range(DH):
                qd = [q_ref[j, 16 * d + 8 * hh:16 * d + 8 * hh + 8, :] for hh in range(2)]
                cur, prev = k_ref[j + 1, 8 * d:8 * d + 8, :], k_ref[j, 8 * d:8 * d + 8, :]
                for w in range(w0, w0 + 4):
                    ks = shifted(prev, cur, w)
                    for hh in range(2):
                        t = qd[hh] * ks[hh]
                        acc[hh][w] = t if d == 0 else acc[hh][w] + t
        probs = []
        for hh in range(2):
            lg = [a * (DH ** -0.5) for a in acc[hh]]
            if first:
                lg = [lg[0]] + [jnp.where(lane >= DIL * w, lg[w], -1e9) for w in range(1, WIN)]
            mx = lg[0]
            for w in range(1, WIN):
                mx = jnp.maximum(mx, lg[w])
            ex = [jnp.exp(t - mx) for t in lg]
            tot = ex[0]
            for w in range(1, WIN):
                tot = tot + ex[w]
            inv = 1.0 / tot
            probs.append([e * inv for e in ex])
        return probs

    def values(j, probs):
        for d in range(DH):
            cur, prev = v_ref[j + 1, 8 * d:8 * d + 8, :], v_ref[j, 8 * d:8 * d + 8, :]
            o = [None, None]
            for w in reversed(range(WIN)):
                vs = shifted(prev, cur, w)
                for hh in range(2):
                    t = probs[hh][w] * vs[hh]
                    o[hh] = t if o[hh] is None else o[hh] + t
            ot_ref[j, 8 * d:8 * d + 8, :] = _words(jnp.concatenate(o, axis=0))

    def keep_history():
        k_ref[0] = k_ref[NT]
        v_ref[0] = v_ref[NT]

    def attn_out(j, zero=None):
        return jnp.dot(_halves(wot_ref[...]), padded(_halves(ot_ref[j]), zero),
                       preferred_element_type=F32)

    def front(b, zero=None):
        transpose_x(b)
        ssm_in((6, 0, 1, 2, 3, 4, 5))
        for j in range(NT):
            proj(b, K, j, zero if j == 0 else None)
            proj(b, Q, j)
            if j:
                proj(b, V, j - 1)
                values(j - 1, p)
            if j < NS:
                scan(j, (3, 0, 1, 2))
            p = scores(j)
        proj(b, V, NT - 1)
        values(NT - 1, p)
        keep_history()

    def finish(b):
        for j in range(NT):
            row = b * TB + 128 * j
            row = row if isinstance(row, int) else pl.multiple_of(row, 128)
            out_ref[pl.ds(row, 128), :] = jnp.concatenate([y_ref[j], attn_out(j)], axis=0).T
        out_copy(b).start()

    for group in groups:
        start(group)
    start(x_copies(1))
    spare_ref[0] = S
    k_ref[0] = jnp.zeros(k_ref.shape[1:], U32)
    wait(groups[0])
    transpose_x(0)
    ssm_in((0,))
    wait(groups[1])
    fr, fi = setup_lambda()
    ssm_in((6, 1, 2, 3))
    scan_block((3, 0))
    wait(groups[2])
    ssm_in((4, 5))
    scan_block((1,))
    setup_w(K)
    wait(groups[3])
    setup_w(Q)
    proj(0, K, 0)
    proj(0, K, 1)
    scan_block((2,))
    wait(groups[4])
    setup_w(V)
    proj(0, Q, 0)
    p0 = scores(0, first=True)
    proj(0, Q, 1)
    p1 = scores(1)
    proj(0, V, 0)
    v_ref[0] = jnp.broadcast_to(v_ref[1][:, 0:1], v_ref.shape[1:])
    values(0, p0)
    proj(0, K, 2)
    proj(0, K, 3)
    wait(groups[5])
    setup_c(fr, fi)
    proj(0, Q, 2)
    p2 = scores(2)
    proj(0, Q, 3)
    p3 = scores(3)
    y_ref[0] = ssm_out(0, 0)
    for j, p in ((1, p1), (2, p2), (3, p3)):
        proj(0, V, j)
        values(j, p)
        y_ref[j] = ssm_out(0, j)
    keep_history()
    setup_wo()

    @pl.loop(1, NB - 1)
    def _(b):
        start(x_copies(b + 1))
        wait(x_copies(b))
        finish(b - 1)
        front(b)
        for j in range(NT):
            y_ref[j] = ssm_out(b, j)

    last = NB - 1
    wait(x_copies(last))
    spare = pl.multiple_of(spare_ref[0], 8)
    stores = [out_copy(b) for b in range(last)]

    def zero_after_start():
        out_ref[S:S + 8, 0:128] = jnp.zeros((8, 128), F32)
        return pltpu.bitcast(out_ref[pl.ds(spare, 8), 0:128], U32)

    def emit(j, lo, hi, t):
        rows, cols = pl.ds(last * TB + 128 * j, 128), pl.ds(lo, hi - lo)
        out_ref[rows, cols] = t.T
        stores.append(pltpu.make_async_copy(out_ref.at[rows, cols], out_hbm.at[rows, cols], osem))
        stores[-1].start()
        return zero_after_start()

    finish(last - 1)
    front(last, zero_after_start())
    sent = [None, None]
    for j in range(NT - 1):
        y_t = ssm_out(last, j)
        sent.append(emit(j, 0, 384, y_t[0:384]))
        ob_t = attn_out(j, sent[-3] if j > 1 else None)
        sent.append(emit(j, 384, 896, jnp.concatenate([y_t[384:D], ob_t], axis=0)))
    j = NT - 1
    ob_t = attn_out(j, sent[-2])
    zero = emit(j, 512, 896, ob_t[64:D])
    emit(j, 0, 384, ssm_out(last, j, 0, 384))
    emit(j, 384, 512, jnp.concatenate([ssm_out(last, j, 384, D, zero), ob_t[0:64]], axis=0))
    wait(stores)


@jax.jit
def pallas_concat_heads__ssm_conv_s5__sliding_local_dilated__prompt_kernel(
    A_x: jax.Array,
    A_Lambda_re: jax.Array,
    A_Lambda_im: jax.Array,
    A_B_re: jax.Array,
    A_B_im: jax.Array,
    A_C_re: jax.Array,
    A_C_im: jax.Array,
    A_log_dt: jax.Array,
    A_Dskip: jax.Array,
    B_x: jax.Array,
    B_wqkv: jax.Array,
    B_wo: jax.Array,
):
    hbm = pl.BlockSpec(memory_space=pltpu.HBM)
    vm = pltpu.VMEM
    out = pl.pallas_call(
        _kernel,
        in_specs=[hbm] * 12,
        out_specs=hbm,
        out_shape=jax.ShapeDtypeStruct((S, 2 * D), F32),
        scratch_shapes=[
            vm((NB, D, TB), BF16), vm((NB, D, TB), BF16),
            vm((D,), BF16), vm((D,), BF16), vm((D,), BF16), vm((D,), BF16),
            vm((D, D), BF16), vm((D, D), BF16), vm((D, D), BF16), vm((D, D), BF16),
            vm((D, 3 * D), BF16), vm((D, D), BF16),
            vm((8, 4, 8, 128), F32),
            vm((8, 8, 128), F32),
            vm((D // 2, 2 * D), U32),
            vm((3 * D // 2, DP), U32),
            vm((D // 2, DP), U32),
            vm((D, 128), F32),
            vm((4, 3 * D // 2, 128), U32),
            vm((4, D // 2, 128), U32),
            vm((TB // 2, D), U32),
            vm((NS, 8, 8 * PITCH, 128), F32),
            vm((NS, 7, 8 * PITCH, 128), F32),
            vm((NT, D, 128), F32),
            vm((NT + 1, D // 2, 128), U32),
            vm((NT + 1, D // 2, 128), U32),
            vm((NT, D // 2, 128), U32),
            vm((NT, D, 128), F32),
            vm((S + 8, 2 * D), F32),
            pltpu.SMEM((1,), jnp.int32),
            pltpu.SemaphoreType.DMA((5 + NB,)),
            pltpu.SemaphoreType.DMA(()),
        ],
        compiler_params=pltpu.CompilerParams(vmem_limit_bytes=64 * 1024 * 1024),
    )(A_x.reshape(S, D).T, B_x.reshape(S, D).T, A_Lambda_re, A_Lambda_im, A_log_dt, A_Dskip,
      A_B_re, A_B_im, A_C_re, A_C_im, B_wqkv, B_wo)
    return out.reshape(1, S, 2 * D)
```
